```python
import jax
import jax.numpy as jnp

def _softmax(x, axis=-1):
    return jax.nn.softmax(x, axis=axis)
def _gelu(x):
    return jax.nn.gelu(x, approximate=True)
def _silu(x):
    return jax.nn.silu(x)
def _sigmoid(x):
    return jax.nn.sigmoid(x)
def _layernorm(x, axis=-1, eps=1e-5):
    m = jnp.mean(x, axis=axis, keepdims=True)
    v = jnp.var(x, axis=axis, keepdims=True)
    return (x - m) / jnp.sqrt(v + eps)
def _scatter_add(tgt, idx, src, axis=0):
    return tgt.at[idx].add(src)
def _segment_sum(src, seg, n):
    return jax.ops.segment_sum(src, seg, n)
class _Rng:
    def __init__(self, key):
        self._k = key
    def _next(self):
        self._k, sub = jax.random.split(self._k)
        return sub
    def normal(self, shape):
        return jax.random.normal(self._next(), shape, dtype=jnp.bfloat16)
    def randint(self, lo, hi, shape):
        return jax.random.randint(self._next(), shape, lo, hi, dtype=jnp.int32)
    def uniform(self, shape, lo=0.0, hi=1.0):
        return jax.random.uniform(self._next(), shape, jnp.bfloat16, lo, hi)
    def permutation(self, n):
        return jax.random.permutation(self._next(), n)


kernel_name = 'interleave_layers__sliding_block_cached__glu_gated_swiglu__decode'

def setup_inputs():
    _rng = _Rng(jax.random.key(int.from_bytes(__import__("os").urandom(4), "little")))
    _w = (lambda a: (lambda t: t.astype(jnp.bfloat16) if jnp.issubdtype(t.dtype, jnp.floating) else t)(jnp.asarray(a)))
    def _A_setup():
        B, Sq, D = 1, 1, 640
        Hq, Hkv, Sk, Dh = 32, 32, 32768, 192
        assert Hq % Hkv == 0, (Hq, Hkv)
        return {
            "x": _w((lambda *s: _rng.normal(s) * 0.05)(B, Sq, D)),
            "k_cache": _w((lambda *s: _rng.normal(s) * 0.05)(B, Hkv, Sk, Dh)),
            "v_cache": _w((lambda *s: _rng.normal(s) * 0.05)(B, Hkv, Sk, Dh)),
            "wq": _w((lambda *s: _rng.normal(s) * 0.05)(D, Hq * Dh) * (D ** -0.5)),
            "wo": _w((lambda *s: _rng.normal(s) * 0.05)(Hq * Dh, D) * ((Hq * Dh) ** -0.5)),
        }
    _A_in = _A_setup()

    def _B_setup():
        B, S, D, F = 1, 1, 640, 1536
        return {
            "x": _w((lambda *s: _rng.normal(s) * 0.05)(B, S, D)),
            "w1": _w((lambda *s: _rng.normal(s) * 0.05)(D, F) * (2.0 / D) ** 0.5),
            "w3": _w((lambda *s: _rng.normal(s) * 0.05)(D, F) * (2.0 / D) ** 0.5),
            "w2": _w((lambda *s: _rng.normal(s) * 0.05)(F, D) * (2.0 / F) ** 0.5),
        }
    _B_in = _B_setup()

    return {
        "A_x": _A_in["x"],
        "A_k_cache": _A_in["k_cache"],
        "A_v_cache": _A_in["v_cache"],
        "A_wq": _A_in["wq"],
        "A_wo": _A_in["wo"],
        "B_x": _B_in["x"],
        "B_w1": _B_in["w1"],
        "B_w3": _B_in["w3"],
        "B_w2": _B_in["w2"],
    }

def reference(A_x, A_k_cache, A_v_cache, A_wq, A_wo, B_x, B_w1, B_w3, B_w2):
    def _A_ref(x, k_cache, v_cache, wq, wo):
        B, Sq, D = x.shape
        Hq, Dh = 32, 192
        Hkv, Sk = k_cache.shape[1], k_cache.shape[2]
        W = min(4096, max(256, Sk // 4))
        rep = Hq // Hkv
        q = (lambda x, *d: x.transpose(*d))((x @ wq).reshape(B, Sq, Hq, Dh), 0, 2, 1, 3)
        k = jnp.repeat(k_cache[:, :, Sk - W:, :], rep, axis=1)
        v = jnp.repeat(v_cache[:, :, Sk - W:, :], rep, axis=1)
        scores = jnp.einsum("bhqd,bhkd->bhqk", q, k) * (Dh ** -0.5)
        p = _softmax(scores, axis=-1)
        o = jnp.einsum("bhqk,bhkd->bhqd", p, v)
        return (lambda x, *d: x.transpose(*d))(o, 0, 2, 1, 3).reshape(B, Sq, Hq * Dh) @ wo

    def _B_ref(x, w1, w3, w2):
        gate = jnp.einsum("bsd,df->bsf", x, w1)
        up = jnp.einsum("bsd,df->bsf", x, w3)
        h = _silu(gate) * up
        out = jnp.einsum("bsf,fd->bsd", h, w2)
        return out

    x = A_x
    x = x + _A_ref(_layernorm(x, axis=-1), A_k_cache, A_v_cache, A_wq, A_wo)
    x = x + _B_ref(_layernorm(x, axis=-1), B_w1, B_w3, B_w2)
    x = x + _A_ref(_layernorm(x, axis=-1), A_k_cache, A_v_cache, A_wq, A_wo)
    x = x + _B_ref(_layernorm(x, axis=-1), B_w1, B_w3, B_w2)
    return x
```

```python
import functools
import numpy as np
import jax
import jax.numpy as jnp
from jax import lax
from jax.experimental import pallas as pl
from jax.experimental.pallas import tpu as pltpu

D, H, DH, SK, F = 640, 32, 192, 32768, 1536
W = min(4096, max(256, SK // 4))
NC = W // 128
C0 = (SK - W) // 128
NG = H // 2
BF, F32, I32 = jnp.bfloat16, jnp.float32, jnp.int32
SCALE = DH ** -0.5
EPS = 1e-5


def _rows16(v):
    return jnp.concatenate([v, v], axis=0).astype(BF)


def _layernorm(x):
    m = jnp.sum(x, axis=-1, keepdims=True) * (1.0 / D)
    c = x - m
    v = jnp.sum(c * c, axis=-1, keepdims=True) * (1.0 / D)
    return c / jnp.sqrt(v + EPS)


def _w(ref, r0, nr, c):
    return pltpu.bitcast(ref[pl.ds(r0, nr), c].reshape(nr * 8, 128), BF)


def _mm(lhs, w):
    return jnp.dot(lhs, w, preferred_element_type=F32)[0:8]


def make_kernel(layers=2, dma=True):
  def kernel(x_ref, k_hbm, v_hbm, wq_hbm, wo_hbm, w1_hbm, w3_hbm, w2_hbm, o_ref,
             ks, vs, wqs, wos, w1s, w3s, w2s, lq, ps, accs, sems):
    def retiled(src, dst, sem):
        d = dst.bitcast(BF)
        return [pltpu.make_async_copy(src.at[:, hf], d.at[:, :, pl.ds(8 * hf, 8), :], sem)
                for hf in range(2)]

    def kv_copy(hbm, buf, g, sem):
        return retiled(hbm.at[pl.ds(24 * g, 24), :, pl.ds(C0, NC)], buf.at[pl.ds(24 * g, 24)], sem)

    k_cp = lambda g: kv_copy(k_hbm, ks, g, sems.at[g % 2])
    v_cp = lambda g: kv_copy(v_hbm, vs, g, sems.at[2 + g % 2])
    wq_cp = lambda: retiled(wq_hbm, wqs, sems.at[4])
    wo_cp = lambda: retiled(wo_hbm, wos, sems.at[5])
    w13_cp = lambda: retiled(w1_hbm, w1s, sems.at[4]) + retiled(w3_hbm, w3s, sems.at[4])
    w2_cp = lambda: retiled(w2_hbm, w2s, sems.at[5])

    def start(cps):
        for c in cps:
            c.start()

    def wait(cps):
        for c in cps:
            c.wait()

    if dma:
        start(wq_cp()); start(k_cp(0)); start(wo_cp())

    sub = lax.broadcasted_iota(I32, (8, 128), 0)
    lane = lax.broadcasted_iota(I32, (8, 128), 1)

    def stage_q(xn, g):
        for t in range(3):
            q = _mm(xn, _w(wqs, 0, D // 16, 3 * g + t))
            head = ((128 * t + lane) >= DH).astype(I32)
            for j in range(4):
                row = jnp.where(sub == 2 * j + head, q, 0.0)
                lq[g % 2, :, pl.ds(128 * (3 * j + t), 128)] = jnp.concatenate(
                    [row, jnp.zeros_like(row)], axis=0).astype(BF)

    def both_halves(op, v):
        v = op(v, pltpu.roll(v, 2, 0))
        return op(v, pltpu.roll(v, 4, 0))

    def stage_s(g):
        lhs = lq[g % 2]
        s = []
        for m in range(NC // 4):
            w = jnp.concatenate([_w(ks, 24 * g, 24, 4 * m + j) for j in range(4)], axis=0)
            s.append(_mm(lhs, w))
        mx = functools.reduce(jnp.maximum, s)
        mx = jnp.max(both_halves(jnp.maximum, mx), axis=-1, keepdims=True)
        e = [jnp.exp((v - mx) * SCALE) for v in s]
        den = jnp.sum(both_halves(jnp.add, functools.reduce(jnp.add, e)), axis=-1, keepdims=True)
        inv = 1.0 / den
        for m in range(NC // 4):
            ps[g % 2, pl.ds(8 * m, 8), :] = e[m] * inv

    def stage_v(g):
        for hh in range(2):
            lo = [None] * 12
            hi = [None] * 12
            for c in range(NC):
                p = jnp.broadcast_to(ps[g % 2, pl.ds(2 * c + hh, 1), :], (8, 128))
                for r in range(12):
                    w = vs[24 * g + 12 * hh + r, c]
                    a = pltpu.bitcast(w << 16, F32) * p
                    b = pltpu.bitcast(w & jnp.int32(-65536), F32) * p
                    lo[r] = a if c == 0 else lo[r] + a
                    hi[r] = b if c == 0 else hi[r] + b
            for r in range(12):
                accs[g % 2, pl.ds(DH * hh + 16 * r, 8, stride=2), :] = lo[r]
                accs[g % 2, pl.ds(DH * hh + 16 * r + 1, 8, stride=2), :] = hi[r]

    def stage_o(g):
        o = []
        for t in range(3):
            a = accs[g % 2, pl.ds(128 * t, 128), :].T
            o.append(jnp.broadcast_to(jnp.sum(a, axis=0, keepdims=True), (8, 128)))
        lhs = _rows16(jnp.concatenate(o, axis=1))
        return jnp.concatenate([_mm(lhs, _w(wos, 24 * g, 24, c)) for c in range(D // 128)], axis=1)

    def layer(l, x):
        first = l == 0

        def on_first(f):
            if dma:
                pl.when(first)(f)

        xn = _rows16(_layernorm(x))

        @on_first
        def _():
            wait(wq_cp())
            start(k_cp(1)); start(v_cp(0))
        stage_q(xn, 0)
        stage_q(xn, 1)

        @on_first
        def _():
            wait(k_cp(0))
            start(k_cp(2)); start(v_cp(1))
        stage_s(0)

        @on_first
        def _():
            wait(wo_cp()); wait(k_cp(1)); wait(v_cp(0))
            start(k_cp(3)); start(v_cp(2))
        stage_q(xn, 2)
        stage_s(1)
        stage_v(0)

        def step(g, x):
            @on_first
            def _():
                wait(k_cp(g + 1)); wait(v_cp(g))

                @pl.when(g + 3 < NG)
                def _():
                    start(k_cp(g + 3))

                @pl.when(g + 2 < NG)
                def _():
                    start(v_cp(g + 2))

                @pl.when(g + 3 == NG)
                def _():
                    start(w13_cp())

                @pl.when(g + 2 == NG)
                def _():
                    start(w2_cp())
            x = x + stage_o(g - 1)
            stage_s(g + 1)
            stage_q(xn, jnp.minimum(g + 2, NG - 1))
            stage_v(g)
            return x

        x = lax.fori_loop(1, NG - 1, step, x)

        @on_first
        def _():
            wait(v_cp(NG - 1))
        x = x + stage_o(NG - 2)
        stage_v(NG - 1)
        x = x + stage_o(NG - 1)

        xn = _rows16(_layernorm(x))

        @on_first
        def _():
            wait(w13_cp())
        hs = []
        for c in range(F // 128):
            gate = _mm(xn, _w(w1s, 0, D // 16, c))
            up = _mm(xn, _w(w3s, 0, D // 16, c))
            hs.append(gate * (1.0 / (1.0 + jnp.exp(-gate))) * up)
        hl = _rows16(jnp.concatenate(hs, axis=1))

        @on_first
        def _():
            wait(w2_cp())
        return x + jnp.concatenate([_mm(hl, _w(w2s, 0, F // 16, c)) for c in range(D // 128)], axis=1)

    x = jnp.broadcast_to(x_ref[0].astype(F32), (8, D))
    x = lax.fori_loop(0, layers, layer, x)
    o_ref[0] = x[0:1].astype(o_ref.dtype)
  return kernel


def build(layers=2, dma=True):
  def f(A_x, A_k_cache, A_v_cache, A_wq, A_wo, B_x, B_w1, B_w3, B_w2):
    def cache_view(c):
        return c.transpose(0, 1, 3, 2).reshape(H * DH // 16, 2, 8, SK // 128, 128).transpose(0, 1, 3, 2, 4)

    def weight_view(w):
        return w.reshape(w.shape[0] // 16, 2, 8, w.shape[1] // 128, 128).transpose(0, 1, 3, 2, 4)

    def tiles(r, c):
        return pltpu.VMEM((r // 16, c // 128, 8, 128), I32)

    ws = (A_wq, A_wo, B_w1, B_w3, B_w2)
    return pl.pallas_call(
        make_kernel(layers, dma),
        out_shape=jax.ShapeDtypeStruct(A_x.shape, A_x.dtype),
        in_specs=[pl.BlockSpec(memory_space=pltpu.VMEM)] + [pl.BlockSpec(memory_space=pl.ANY)] * 7,
        out_specs=pl.BlockSpec(memory_space=pltpu.VMEM),
        scratch_shapes=[tiles(H * DH, W), tiles(H * DH, W)] + [tiles(*w.shape) for w in ws] + [
            pltpu.VMEM((2, 16, 1536), BF),
            pltpu.VMEM((2, 2 * NC, 128), F32),
            pltpu.VMEM((2, 2 * DH, 128), F32),
            pltpu.SemaphoreType.DMA((6,)),
        ],
        compiler_params=pltpu.CompilerParams(vmem_limit_bytes=127 * 2**20),
        name=f"fused_{layers}_{int(dma)}",
    )(A_x, cache_view(A_k_cache), cache_view(A_v_cache), *[weight_view(w) for w in ws])
  return f


@jax.jit
def pallas_interleave_layers__sliding_block_cached__glu_gated_swiglu__decode_kernel(
    A_x: jax.Array,
    A_k_cache: jax.Array,
    A_v_cache: jax.Array,
    A_wq: jax.Array,
    A_wo: jax.Array,
    B_x: jax.Array,
    B_w1: jax.Array,
    B_w3: jax.Array,
    B_w2: jax.Array,
):
    return build()(A_x, A_k_cache, A_v_cache, A_wq, A_wo, B_x, B_w1, B_w3, B_w2)
```

```python
import functools
import numpy as np
import jax
import jax.numpy as jnp
from jax import lax
from jax.experimental import pallas as pl
from jax.experimental.pallas import tpu as pltpu

D, H, DH, SK, F = 640, 32, 192, 32768, 1536
W = min(4096, max(256, SK // 4))
NC = W // 128
C0 = (SK - W) // 128
NG = H // 2
BF, F32, I32 = jnp.bfloat16, jnp.float32, jnp.int32
SCALE = DH ** -0.5
EPS = 1e-5


def _rows16(v):
    return jnp.concatenate([v, v], axis=0).astype(BF)


def _layernorm(x):
    m = jnp.sum(x, axis=-1, keepdims=True) * (1.0 / D)
    c = x - m
    v = jnp.sum(c * c, axis=-1, keepdims=True) * (1.0 / D)
    return c / jnp.sqrt(v + EPS)


def _w(ref, r0, nr, c):
    return pltpu.bitcast(ref[pl.ds(r0, nr), c].reshape(nr * 8, 128), BF)


def _mm(lhs, w):
    return jnp.dot(lhs, w, preferred_element_type=F32)[0:8]


def make_kernel(layers=2, dma=True, rg=4, cgran=8, extra=0, w2split=(0, 10, 12), sord=2, lag=6, tstep=4, ft=.5, f0=-.02, f1=.68, f2=.78, f3=.88):
  def kernel(x_hbm, k_hbm, v_hbm, wq_hbm, wo_hbm, w1_hbm, w3_hbm, w2_hbm, o_ref,
             ks, vs, wqs, wos, w1s, w3s, w2s, x_ref, lq, lo_buf, accs, dens, sems, *ps):
    def retiled(src, dst, sem):
        d = dst.bitcast(BF)
        return [pltpu.make_async_copy(src.at[:, hf], d.at[:, :, pl.ds(8 * hf, 8), :], sem)
                for hf in range(2)]

    def kv_copy(hbm, buf, g, sem):
        return retiled(hbm.at[pl.ds(24 * g, 24), :, pl.ds(C0, NC)], buf.at[pl.ds(24 * g, 24)], sem)

    k_cp = lambda g: kv_copy(k_hbm, ks, g, sems.at[g % 2])
    v_cp = lambda g: kv_copy(v_hbm, vs, g, sems.at[2 + g % 2])
    wq_cp = lambda: retiled(wq_hbm, wqs, sems.at[4])
    wo_cp = lambda: retiled(wo_hbm, wos, sems.at[5])
    w13_cp = lambda: retiled(w1_hbm, w1s, sems.at[4]) + retiled(w3_hbm, w3s, sems.at[4])
    W2S = w2split
    w2_sem = [5, 0, 1, 2]
    w2_cp = lambda i: retiled(w2_hbm.at[pl.ds(8 * W2S[i], 8 * (W2S[i + 1] - W2S[i]))],
                              w2s.at[pl.ds(8 * W2S[i], 8 * (W2S[i + 1] - W2S[i]))], sems.at[w2_sem[i]])

    def start(cps):
        for c in cps:
            c.start()

    def wait(cps):
        for c in cps:
            c.wait()

    if dma:
        x_cp = pltpu.make_async_copy(x_hbm, x_ref, sems.at[3])
        start(wq_cp()); x_cp.start(); start(k_cp(0)); start(wo_cp())
        x_cp.wait()

    sub = lax.broadcasted_iota(I32, (8, 128), 0)
    lane = lax.broadcasted_iota(I32, (8, 128), 1)

    LQ, LX, LO, LJ = 0, 12, 17, 20

    unit = [None]
    NP = NC // cgran

    def tie(v, lag=lag):
        if unit[0] is not None:
            ps[(unit[0] + lag) % NP][2 * cgran] = v

    def put(i, v):
        buf = lo_buf if LO <= i < LJ else lq
        buf[pl.ds(8 * i, 8), :] = pltpu.bitcast(v, I32)

    def lhs(i, g):
        buf = lo_buf if LO <= i < LJ else lq
        return pltpu.bitcast(buf[pl.ds(pl.multiple_of(8 * i + 8 * (g >> 8), 8), 8), :], BF)

    def stage_q(g, out):
        for kk in range(D // 128):
            for t in range(3):
                y = _mm(lhs(LX + kk, g), _w(wqs, 8 * kk, 8, 3 * g + t))
                if kk == 0:
                    out.append(y)
                else:
                    out[t] = out[t] + y
                tie(out[t])
                yield

    def store_q(qs):
        for t, q in enumerate(qs):
            head = ((128 * t + lane) >= DH).astype(I32)
            for j in range(4):
                row = jnp.where(sub == 2 * j + head, q, 0.0)
                put(LQ + 3 * j + t, jnp.concatenate([row, jnp.zeros_like(row)], axis=0).astype(BF))

    def both_halves(op, v):
        v = op(v, pltpu.roll(v, 2, 0))
        return op(v, pltpu.roll(v, 4, 0))

    def stage_s(g, out):
        s = [None] * (NC // 4)
        if sord == 0:
            order = [(j, t, m) for j in range(4) for t in range(3) for m in range(NC // 4)]
        elif sord == 1:
            order = [(2 * j1 + j0, t, m) for j1 in range(2) for t in range(3) for m in range(NC // 4) for j0 in range(2)]
        else:
            order = [(j, t, m) for m in range(NC // 4) for t in range(3) for j in range(4)]
        for j, t, m in order:
            y = _mm(lhs(LQ + 3 * j + t, g), _w(ks, 24 * g + 8 * t, 8, 4 * m + j))
            s[m] = y if s[m] is None else s[m] + y
            tie(s[m])
            yield
        out.extend(s)

    def stage_p(s, g):
        mx = functools.reduce(jnp.maximum, s)
        mx = jnp.max(both_halves(jnp.maximum, mx), axis=-1, keepdims=True)
        e = [jnp.exp((v - mx) * SCALE) for v in s]
        for m in range(NC // 4):
            for i in range(8):
                ps[(8 * m + i) // (2 * cgran)][(8 * m + i) % (2 * cgran)] = jnp.broadcast_to(e[m][i:i + 1], (8, 128))
        dens[g % 4] = both_halves(jnp.add, functools.reduce(jnp.add, e))

    def stage_v(g):
        for hh in range(2):
            for r0 in range(0, 12, rg):
                lo = [None] * rg
                hi = [None] * rg
                for c in range(NC):
                    p = ps[c // cgran][2 * (c % cgran) + hh + (g >> 8)]
                    for r in range(rg):
                        w = vs[24 * g + 12 * hh + r0 + r, c]
                        a = pltpu.bitcast(w << 16, F32) * p
                        b = pltpu.bitcast(w & jnp.int32(-65536), F32) * p
                        lo[r] = a if c == 0 else lo[r] + a
                        hi[r] = b if c == 0 else hi[r] + b
                    if c % cgran == cgran - 1:
                        for i, v in enumerate((lo + hi)[::tstep]):
                            put(LJ + i, v)
                        lo_buf[pl.ds(0, 8), :] = pltpu.bitcast(lo[0], I32)
                        unit[0] += 1
                        yield
                for r in range(rg):
                    accs[pl.ds(DH * hh + 16 * (r0 + r), 8, stride=2), :] = lo[r]
                    accs[pl.ds(DH * hh + 16 * (r0 + r) + 1, 8, stride=2), :] = hi[r]

    def stage_t(g):
        inv = 1.0 / jnp.sum(dens[g % 4], axis=-1, keepdims=True)
        inv0 = jnp.broadcast_to(inv[0:1], (8, 128))
        inv1 = jnp.broadcast_to(inv[1:2], (8, 128))
        blocks = [accs[pl.ds(128 * t, 128), :] for t in range(3)]
        yield
        for t in range(3):
            o = jnp.broadcast_to(jnp.sum(blocks[t].T, axis=0, keepdims=True), (8, 128))
            o = o * jnp.where(128 * t + lane >= DH, inv1, inv0)
            put(LO + t, _rows16(o))
            tie(o, NP - 1)
            yield

    def stage_o(g, xs):
        for t in range(3):
            for c in range(D // 128):
                xs[c] = xs[c] + _mm(lhs(LO + t, g), _w(wos, 24 * g + 8 * t, 8, c))
                tie(xs[c])
                yield

    def run(*gens):
        for gen in gens:
            for _ in gen:
                pass

    def mix(*streams):
        ev = []
        unit[0] = 0
        for i, (gen, n, t0, t1) in enumerate(streams):
            ev += [(t0 + (t1 - t0) * (k + 0.5) / n, i) for k in range(n)] + [(t1 + 1e-9, i)]
        for _, i in sorted(ev):
            next(streams[i][0], None)
        unit[0] = None

    def split(x):
        return [x[:, 128 * c:128 * (c + 1)] for c in range(D // 128)]

    def layer(l, x):
        first = l == 0

        def on_first(f):
            if dma:
                pl.when(first)(f)

        xn = _rows16(_layernorm(x))
        for kk in range(D // 128):
            put(LX + kk, xn[:, 128 * kk:128 * (kk + 1)])

        @on_first
        def _():
            wait(wq_cp())
            start(k_cp(1)); start(v_cp(0))
            wait(k_cp(0))
            start(k_cp(2)); start(v_cp(1))
        z = l >> 8
        s, q = [], []
        run(stage_q(z, q))
        store_q(q)
        q = []
        run(stage_s(z, s), stage_q(z + 1, q))
        stage_p(s, 0)
        store_q(q)
        nv = 2 * NC * 12 // (rg * cgran)

        @on_first
        def _():
            wait(wo_cp()); wait(k_cp(1)); wait(v_cp(0))
            start(k_cp(3)); start(v_cp(2))
        s, q = [], []
        mix((stage_s(z + 1, s), 96, 0, f1), (stage_q(z + 2, q), 15, f1, f2), (stage_v(z), nv, 0, 1))
        stage_p(s, 1)
        store_q(q)

        def step(g, x):
            @on_first
            def _():
                wait(k_cp(g + 1)); wait(v_cp(g))

                @pl.when(g + 3 < NG)
                def _():
                    start(k_cp(g + 3))

                @pl.when(g + 2 < NG)
                def _():
                    start(v_cp(g + 2))

                @pl.when(g + 3 == NG)
                def _():
                    start(w13_cp())

                @pl.when(g + 2 == NG)
                def _():
                    start(w2_cp(0))
            xs = split(x)
            s, q = [], []
            mix((stage_t(g - 1), 4, -ft / 4, ft), (stage_s(g + 1, s), 96, f0, f1),
                (stage_q(jnp.minimum(g + 2, NG - 1), q), 15, f1, f2),
                (stage_o(g - 1, xs), 15, f2, f3), (stage_v(g), nv, 0, 1))
            stage_p(s, g + 1)
            store_q(q)
            return jnp.concatenate(xs, axis=1)

        if extra:
            x = lax.fori_loop(1, NG - 1 + extra * l, lambda i, x: step(jnp.minimum(i, NG - 2), x), x)
        else:
            x = lax.fori_loop(1, NG - 1, step, x)

        @on_first
        def _():
            wait(v_cp(NG - 1))
            for i in range(1, len(W2S) - 1):
                start(w2_cp(i))
        xs = split(x)
        mix((stage_t(NG - 2), 4, -.1, .4), (stage_o(z + NG - 2, xs), 15, .5, .8), (stage_v(z + NG - 1), nv, 0, 1))
        run(stage_t(NG - 1), stage_o(z + NG - 1, xs))
        x = jnp.concatenate(xs, axis=1)

        xn = _rows16(_layernorm(x))

        @on_first
        def _():
            wait(w13_cp())
        hs = []
        for c in range(F // 128):
            gate = _mm(xn, _w(w1s, 0, D // 16, c))
            up = _mm(xn, _w(w3s, 0, D // 16, c))
            hs.append(gate * (1.0 / (1.0 + jnp.exp(-gate))) * up)
        hl = _rows16(jnp.concatenate(hs, axis=1))

        xs = split(x)
        for i in range(len(W2S) - 1):
            on_first(lambda: wait(w2_cp(i)))
            for kk in range(W2S[i], W2S[i + 1]):
                for c in range(D // 128):
                    xs[c] = xs[c] + _mm(hl[:, 128 * kk:128 * (kk + 1)], _w(w2s, 8 * kk, 8, c))
        return jnp.concatenate(xs, axis=1)

    x = jnp.broadcast_to(x_ref[0].astype(F32), (8, D))
    x = lax.fori_loop(0, layers, layer, x)
    o_ref[0] = x[0:1].astype(o_ref.dtype)
  return kernel


def build(layers=2, dma=True, flags=None, cgran=4, **kw):
  def f(A_x, A_k_cache, A_v_cache, A_wq, A_wo, B_x, B_w1, B_w3, B_w2):
    def cache_view(c):
        return c.transpose(0, 1, 3, 2).reshape(H * DH // 16, 2, 8, SK // 128, 128).transpose(0, 1, 3, 2, 4)

    def weight_view(w):
        return w.reshape(w.shape[0] // 16, 2, 8, w.shape[1] // 128, 128).transpose(0, 1, 3, 2, 4)

    def tiles(r, c):
        return pltpu.VMEM((r // 16, c // 128, 8, 128), I32)

    ws = (A_wq, A_wo, B_w1, B_w3, B_w2)
    return pl.pallas_call(
        make_kernel(layers, dma, cgran=cgran, **kw),
        out_shape=jax.ShapeDtypeStruct(A_x.shape, A_x.dtype),
        in_specs=[pl.BlockSpec(memory_space=pl.ANY)] * 8,
        out_specs=pl.BlockSpec(memory_space=pltpu.VMEM),
        scratch_shapes=[tiles(H * DH, W), tiles(H * DH, W)] + [tiles(*w.shape) for w in ws] + [
            pltpu.VMEM(A_x.shape, A_x.dtype),
            pltpu.VMEM((8 * 44, 128), I32),
            pltpu.VMEM((8 * 20, 128), I32),
            pltpu.VMEM((2 * DH, 128), F32),
            pltpu.VMEM((4, 8, 128), F32),
            pltpu.SemaphoreType.DMA((6,)),
        ] + [pltpu.VMEM((2 * cgran + 1, 8, 128), F32)] * (NC // cgran),
        compiler_params=pltpu.CompilerParams(vmem_limit_bytes=127 * 2**20, flags=flags),
        name=f"fused_{layers}_{int(dma)}",
    )(A_x, cache_view(A_k_cache), cache_view(A_v_cache), *[weight_view(w) for w in ws])
  return f


@jax.jit
def pallas_interleave_layers__sliding_block_cached__glu_gated_swiglu__decode_kernel(
    A_x: jax.Array,
    A_k_cache: jax.Array,
    A_v_cache: jax.Array,
    A_wq: jax.Array,
    A_wo: jax.Array,
    B_x: jax.Array,
    B_w1: jax.Array,
    B_w3: jax.Array,
    B_w2: jax.Array,
):
    return build()(A_x, A_k_cache, A_v_cache, A_wq, A_wo, B_x, B_w1, B_w3, B_w2)
```

```python
import functools
import jax
import jax.numpy as jnp
from jax import lax
from jax.experimental import pallas as pl
from jax.experimental.pallas import tpu as pltpu

D, H, DH, SK, F = 640, 32, 192, 32768, 1536
W = min(4096, max(256, SK // 4))
NC = W // 128
C0 = (SK - W) // 128
NG = H // 2
NT = H * DH // 16
ND = D // 128
BF, F32, I32 = jnp.bfloat16, jnp.float32, jnp.int32
SCALE = DH ** -0.5
EPS = 1e-5


def _rows16(v):
    return jnp.concatenate([v, v], axis=0).astype(BF)


def _rows8(v):
    return jnp.concatenate([v, jnp.zeros_like(v)], axis=0).astype(BF)


def _layernorm(x):
    c = x - jnp.sum(x, axis=-1, keepdims=True) * (1.0 / D)
    v = jnp.sum(c * c, axis=-1, keepdims=True) * (1.0 / D)
    return c, jnp.broadcast_to(1.0 / jnp.sqrt(v + EPS), (8, 128))


def _w(ref, r0, c):
    return pltpu.bitcast(ref[pl.ds(r0, 8), c].reshape(64, 128), BF)


def _mm(lhs, w):
    return jnp.dot(lhs, w, preferred_element_type=F32)[0:8]


def _halves(w):
    return pltpu.bitcast(w << 16, F32), pltpu.bitcast(w & jnp.int32(-65536), F32)


def make_kernel(layers=2, extra=0, cgran=4, nx=0, ne=0, nxl=12, rg=4, lag=6, tstep=4, ktie=False, sord=2,
                f0=-.02, f3=.88, ft0=-.05, ft=.46, tlag=1.0, fp=None, fl=.85, w2split=(0, 8, 12), sstore=True):
  NV = NC - nx
  NP = -(-NV // cgran)
  w2_sem = [5, 0, 1, 2]
  echunks = [int((i + 0.5) * NV / ne) for i in range(ne)]

  def kernel(x_hbm, k_hbm, v_hbm, wq_hbm, wo_hbm, w1_hbm, w3_hbm, w2_hbm, o_ref,
             ks, vs, ve, wqs, wos, w1s, w3s, w2s, xs, lq, lo_buf, accs, accx, dens, masks, sems, *ps):
    *ps, x_ref = ps
    def retiled(src, dst, sem):
        d = dst.bitcast(BF)
        return [pltpu.make_async_copy(src.at[:, hf], d.at[:, :, pl.ds(8 * hf, 8), :], sem)
                for hf in range(2)]

    def kv_copy(hbm, buf, g, sem):
        return retiled(hbm.at[pl.ds(24 * g, 24), :, pl.ds(C0, NC)], buf.at[pl.ds(24 * g, 24)], sem)

    k_cp = lambda g: kv_copy(k_hbm, ks, g, sems.at[g & 1])
    v_cp = lambda g: kv_copy(v_hbm, vs, g, sems.at[2 + (g & 1)])
    wq_cp = lambda: retiled(wq_hbm, wqs.at[pl.ds(0, D // 16)], sems.at[4])
    wo_cp = lambda: retiled(wo_hbm, wos.at[pl.ds(0, NT)], sems.at[5])
    w13_cp = lambda: retiled(w1_hbm, w1s, sems.at[4]) + retiled(w3_hbm, w3s, sems.at[4])

    def w2_cp(i):
        rows = pl.ds(8 * w2split[i], 8 * (w2split[i + 1] - w2split[i]))
        return retiled(w2_hbm.at[rows], w2s.at[rows], sems.at[w2_sem[i]])

    def start(cps):
        for c in cps:
            c.start()

    def wait(cps):
        for c in cps:
            c.wait()

    x_cp = pltpu.make_async_copy(x_hbm, x_ref, sems.at[3])
    start(wq_cp()); x_cp.start(); start(k_cp(0)); start(wo_cp())

    sub = lax.broadcasted_iota(I32, (8, 128), 0)
    lane = lax.broadcasted_iota(I32, (8, 128), 1)
    for t in range(3):
        for j in range(4):
            masks[3 * j + t] = jnp.where(sub == j, jnp.where(128 * t + lane >= DH, -65536, 65535), 0)
    x_cp.wait()

    LQ, LX, LS, LJ, LP, LO = 0, 12, 17, 18, 42, 44
    unit = [None, True]

    def tie(v, lag=lag):
        if unit[0] is not None and unit[1]:
            ps[(unit[0] + lag) % NP][2 * cgran] = v

    def put(buf, i, v):
        buf[i] = pltpu.bitcast(v, I32)

    def get(buf, i, g, dtype=BF):
        return pltpu.bitcast(buf[i + 4 * (g >> 8)], dtype)

    def stage_q(g, out):
        for kk in range(ND):
            for t in range(3):
                y = _mm(get(lq, LX + kk, g), _w(wqs, 8 * kk, 3 * g + t))
                if kk == 0:
                    out.append(y)
                else:
                    out[t] = out[t] + y
                tie(out[t])
                yield

    def store_q(qs):
        for t, q in enumerate(qs):
            q = pltpu.bitcast(_rows16(q * pltpu.bitcast(lq[LS], F32)), I32)
            for j in range(4):
                lq[LQ + 3 * j + t] = q & masks[3 * j + t]

    def both_halves(op, v):
        v = op(v, pltpu.roll(v, 2, 0))
        return op(v, pltpu.roll(v, 4, 0))

    def stage_s(g, s):
        s.extend([None] * (NC // 4))
        if sord == 1:
            order = [(2 * j1 + j0, t, m) for m in range(NC // 4) for j1 in range(2) for t in range(3) for j0 in range(2)]
        elif sord == 2:
            order = [(j, t, m) for m in range(NC // 4) for t in range(3) for j in range(4)]
        else:
            order = [(j, t, m + mm) for m in range(0, NC // 4, 2) for t in range(3) for j in range(4) for mm in range(2)]
        for j, t, m in order:
            y = _mm(get(lq, LQ + 3 * j + t, g), _w(ks, 24 * g + 8 * t, 4 * m + j))
            s[m] = y if s[m] is None else s[m] + y
            tie(s[m])
            yield

    def stage_p(s, g):
        mx = functools.reduce(jnp.maximum, s)
        mx = jnp.max(both_halves(jnp.maximum, mx), axis=-1, keepdims=True)
        e = [jnp.exp((v - mx) * SCALE) for v in s]
        for c in range(NC):
            m, j = divmod(c, 4)
            if c >= NV:
                put(lq, LP + c - NV, _rows8(jnp.where(sub // 2 == j, e[m], 0.0)))
                continue
            for hh in range(2):
                ps[c // cgran][2 * (c % cgran) + hh] = jnp.broadcast_to(e[m][2 * j + hh:2 * j + hh + 1], (8, 128))
        dens[g & 3] = both_halves(jnp.add, functools.reduce(jnp.add, e))

    def expand(g):
        def body(r, _):
            for i, c in enumerate(echunks):
                lo, hi = _halves(vs[24 * g + r, c])
                vs[24 * g + r, c] = pltpu.bitcast(lo, I32)
                ve[24 * g + r, i] = hi
        if ne:
            lax.fori_loop(0, 24, body, None)

    def stage_v(g, chunks, switch):
        for hh in range(2):
            for r0 in range(0, 12, rg):
                acc = [None] * (2 * rg)
                for c in chunks:
                    p = ps[c // cgran][2 * (c % cgran) + hh + 4 * (g >> 8)]
                    for r in range(rg):
                        row = 24 * g + 12 * hh + r0 + r
                        if c in echunks:
                            parts = pltpu.bitcast(vs[row, c], F32), ve[row, echunks.index(c)]
                        else:
                            parts = _halves(vs[row, c])
                        for i in range(2):
                            a = parts[i] * p
                            acc[rg * i + r] = a if c == chunks[0] else acc[rg * i + r] + a
                    if c % cgran == cgran - 1 or c == chunks[-1]:
                        for bufs in switch():
                            if bufs[1] is None:
                                for i, v in enumerate(acc[::tstep]):
                                    put(bufs[0], LJ + i, v)
                            else:
                                bufs[0][bufs[1], 0] = pltpu.bitcast(acc[-1], I32)
                        unit[0] += 1
                        yield
                for r in range(rg):
                    for i in range(2):
                        accs[pl.ds(DH * hh + 16 * (r0 + r) + i, 8, stride=2), :] = acc[rg * i + r]

    def stage_x(g, chunks):
        acc = [jnp.zeros((8, 128), F32)] * 3
        for n, c in enumerate(chunks):
            for t in range(3):
                y = lax.dot_general(get(lq, LP + c - NV + (NC if c < NV else 0), g), _w(vs, 24 * g + 8 * t, c),
                                    (((1,), (1,)), ((), ())), preferred_element_type=F32)[0:8]
                acc[t] = y if n == 0 else acc[t] + y
                tie(acc[t])
                yield
        for t in range(3 if chunks else 0):
            accx[t] = jnp.where((sub & 1) == (128 * t + lane >= DH).astype(I32), acc[t], 0.0)

    def stage_t(g, with_x):
        inv = 1.0 / jnp.sum(dens[g & 3], axis=-1, keepdims=True)
        inv0 = jnp.broadcast_to(inv[0:1], (8, 128))
        inv1 = jnp.broadcast_to(inv[1:2], (8, 128))
        for t in range(3):
            blk = accs[pl.ds(pl.multiple_of(128 * t + 128 * (g >> 8), 128), 128), :]
            o = jnp.sum(blk.T.reshape(16, 8, 128), axis=0)
            if with_x:
                o = o + accx[t]
            o = jnp.broadcast_to(jnp.sum(o, axis=0, keepdims=True), (8, 128))
            o = o * (inv0, jnp.where(lane >= DH - 128, inv1, inv0), inv1)[t]
            put(lo_buf, LO + t, _rows16(o))
            tie(o, min(NP - 1, int(tlag * NP)))
            yield

    def stage_o(g):
        acc = [xs[c + 8 * (g >> 8)] for c in range(ND)]
        for t in range(3):
            for c in range(ND):
                acc[c] = acc[c] + _mm(get(lo_buf, LO + t, g), _w(wos, 24 * g + 8 * t, c))
                tie(acc[c])
                yield
        for c in range(ND):
            xs[c] = acc[c]

    def run(*gens):
        for gen in gens:
            for _ in gen:
                pass

    def mix(mxu, side, g, chunks, f0=f0, f3=f3, back=True):
        nv = 2 * (12 // rg) * len({c // cgran for c in chunks})
        tot = sum(n * cost for _, n, cost, _, _ in mxu)
        ev, gens, pos = [], [], 0
        for gen, n, cost, lbuf, wbuf in mxu:
            for k in range(n):
                ev.append((f0 + (f3 - f0) * (pos + 0.5 * cost) / tot, len(gens), lbuf, wbuf))
                pos += cost
            ev.append((f0 + (f3 - f0) * pos / tot - 1e-9, len(gens), None, None))
            gens.append(gen)
        for gen, n, t0, t1 in side:
            ev += [(t0 + (t1 - t0) * (k + 0.5) / n, len(gens), None, None) for k in range(n)]
            gens.append(gen)
        ev += [((k + 0.5) / nv, len(gens), None, None) for k in range(nv)] + [(2, len(gens), None, None)]
        ev.sort(key=lambda e: e[:2])
        now = [0]

        def switch():
            out = {}
            for e in ev[now[0] + 1:]:
                if e[1] == len(gens) - 1:
                    break
                if e[2] is not None:
                    out[id(e[2])] = (e[2], None)
                if e[3] is not None and ktie:
                    out[id(e[3][0])] = e[3]
            return list(out.values())

        gens.append(stage_v(g, chunks, switch))
        unit[:] = 0, back
        for now[0], e in enumerate(ev):
            next(gens[e[1]], None)
        unit[0] = None

    def get_x():
        return jnp.concatenate([xs[c] for c in range(ND)], axis=1)

    v_chunks, x_chunks = list(range(NV)), list(range(NV, NC))

    def attend(g, with_o):
        s, q = [], []
        mxu = [(stage_s(g + 1, s), 96, 1, lq, (ks, NT)), (stage_x(g, x_chunks), 3 * nx, 2, lq, None),
               (stage_q(jnp.minimum(g + 2, NG - 1), q), 15, 1, lq, (wqs, D // 16))]
        side = []
        if with_o:
            mxu.append((stage_o(g - 1), 15, 1, lo_buf, (wos, NT)))
            side.append((stage_t(g - 1, nx > 0), 3, ft0, ft))
        mix(mxu, side, g, v_chunks)
        stage_p(s, g + 1)
        store_q(q)

    def layer(l, _):
        on_first = pl.when(l == 0)
        z = l >> 8

        @on_first
        def _():
            wait(wq_cp())
            start(k_cp(1)); start(v_cp(0))
            wait(k_cp(0))
            start(k_cp(2)); start(v_cp(1))
        xc, rstd = _layernorm(get_x())
        xc = _rows16(xc)
        for kk in range(ND):
            put(lq, LX + kk, xc[:, 128 * kk:128 * (kk + 1)])
        put(lq, LS, rstd)
        s, q = [], []
        run(stage_q(z, q))
        store_q(q)
        q = []
        run(stage_s(z, s), stage_q(z + 1, q))
        stage_p(s, 0)
        store_q(q)

        @on_first
        def _():
            wait(wo_cp()); wait(k_cp(1)); wait(v_cp(0))
            start(k_cp(3)); start(v_cp(2))
            expand(0)
        attend(z, False)

        def step(g, _):
            g = jnp.minimum(g, NG - 2) if extra else g

            @on_first
            def _():
                wait(k_cp(g + 1)); wait(v_cp(g))

                @pl.when(g + 3 < NG)
                def _():
                    start(k_cp(g + 3))

                @pl.when(g + 2 < NG)
                def _():
                    start(v_cp(g + 2))

                @pl.when(g + 3 == NG)
                def _():
                    start(w13_cp())

                @pl.when(g + 2 == NG)
                def _():
                    start(w2_cp(0))
                expand(g)
            attend(g, True)

        lax.fori_loop(1, NG - 1 + (extra * l if extra else 0), step, None)

        @on_first
        def _():
            wait(v_cp(NG - 1))
            for i in range(1, len(w2split) - 1):
                start(w2_cp(i))
            expand(NG - 1)
            wait(w13_cp())
        moved = [c for c in reversed(v_chunks) if c not in echunks][:nxl]
        for c in moved:
            p0, p1 = (ps[c // cgran][2 * (c % cgran) + hh] for hh in range(2))
            put(lq, LP + c - NV + NC, _rows8(jnp.where(sub == 0, p0, jnp.where(sub == 1, p1, 0.0))))
        t = stage_t(z + NG - 2, nx > 0)
        mix([(stage_x(z + NG - 1, x_chunks + moved), 3 * (nx + nxl), 2, lq, None),
             (stage_o(z + NG - 2), 15, 1, lo_buf, (wos, NT))],
            [(t, 3, ft0, ft)], z + NG - 1, [c for c in v_chunks if c not in moved], f3=fl, back=False)
        run(stage_t(z + NG - 1, nx + nxl > 0), stage_o(z + NG - 1))

        on_first(lambda: wait(w2_cp(0)))
        x = get_x()
        xc, rstd = _layernorm(x)
        xc = _rows16(xc)
        hs = []
        for c in range(F // 128):
            gate, up = (rstd * functools.reduce(jnp.add, [
                _mm(xc[:, 128 * kk:128 * (kk + 1)], _w(w, 8 * kk, c)) for kk in range(ND)]) for w in (w1s, w3s))
            hs.append(_rows16(gate * (1.0 / (1.0 + jnp.exp(-gate))) * up))
        acc = [x[:, 128 * c:128 * (c + 1)] for c in range(ND)]
        for i in range(len(w2split) - 1):
            if i:
                on_first(lambda: wait(w2_cp(i)))
            for kk in range(w2split[i], w2split[i + 1]):
                for c in range(ND):
                    acc[c] = acc[c] + _mm(hs[kk], _w(w2s, 8 * kk, c))
        for c in range(ND):
            xs[c] = acc[c]

    x = jnp.broadcast_to(x_ref[0].astype(F32), (8, D))
    for c in range(ND):
        xs[c] = x[:, 128 * c:128 * (c + 1)]
    lax.fori_loop(0, layers, layer, None)
    o_ref[0] = get_x()[0:1].astype(o_ref.dtype)

  def tiles(r, c, pad=0):
      return pltpu.VMEM((r // 16 + pad, c // 128, 8, 128), I32)

  def vregs(n, dtype):
      return pltpu.VMEM((-(-n // 4) * 4, 8, 128), dtype)

  scratch = [
      tiles(H * DH, W, 1), tiles(H * DH, W), pltpu.VMEM((NT, max(ne, 1), 8, 128), F32),
      tiles(D, H * DH, 1), tiles(H * DH, D, 4), tiles(D, F), tiles(D, F), tiles(F, D),
      vregs(8, F32), vregs(42 + NC, I32), vregs(48, I32),
      pltpu.VMEM((2 * DH, 128), F32), vregs(4, F32), vregs(4, F32), vregs(12, I32),
      pltpu.SemaphoreType.DMA((6,)),
  ] + [vregs(2 * cgran + 1, F32)] * NP + [pltpu.VMEM((1, 1, D), BF)]
  return kernel, scratch


def build(flags=None, **kw):
  def f(A_x, A_k_cache, A_v_cache, A_wq, A_wo, B_x, B_w1, B_w3, B_w2):
    def cache_view(c):
        return c.transpose(0, 1, 3, 2).reshape(NT, 2, 8, SK // 128, 128).transpose(0, 1, 3, 2, 4)

    def weight_view(w):
        return w.reshape(w.shape[0] // 16, 2, 8, w.shape[1] // 128, 128).transpose(0, 1, 3, 2, 4)

    kernel, scratch = make_kernel(**kw)
    return pl.pallas_call(
        kernel,
        out_shape=jax.ShapeDtypeStruct(A_x.shape, A_x.dtype),
        in_specs=[pl.BlockSpec(memory_space=pl.ANY)] * 8,
        out_specs=pl.BlockSpec(memory_space=pltpu.VMEM),
        scratch_shapes=scratch,
        compiler_params=pltpu.CompilerParams(vmem_limit_bytes=128 * 2**20, flags=flags),
        name="fused",
    )(A_x, cache_view(A_k_cache), cache_view(A_v_cache),
      *[weight_view(w) for w in (A_wq, A_wo, B_w1, B_w3, B_w2)])
  return f


@jax.jit
def pallas_interleave_layers__sliding_block_cached__glu_gated_swiglu__decode_kernel(
    A_x: jax.Array,
    A_k_cache: jax.Array,
    A_v_cache: jax.Array,
    A_wq: jax.Array,
    A_wo: jax.Array,
    B_x: jax.Array,
    B_w1: jax.Array,
    B_w3: jax.Array,
    B_w2: jax.Array,
):
    return build(**dict(nx=2,cgran=5,rg=4,lag=5,ne=6,nxl=13,tstep=2,sord=2,f3=.88,ft0=-.05,ft=.36))(A_x, A_k_cache, A_v_cache, A_wq, A_wo, B_x, B_w1, B_w3, B_w2)
```

```python
import functools
import jax
import jax.numpy as jnp
from jax import lax
from jax.experimental import pallas as pl
from jax.experimental.pallas import tpu as pltpu

D, H, DH, SK, F = 640, 32, 192, 32768, 1536
W = min(4096, max(256, SK // 4))
NC = W // 128
C0 = (SK - W) // 128
NG = H // 2
NT = H * DH // 16
ND = D // 128
BF, F32, I32 = jnp.bfloat16, jnp.float32, jnp.int32
SCALE = DH ** -0.5
EPS = 1e-5


def _rows16(v):
    return jnp.concatenate([v, v], axis=0).astype(BF)


def _rows8(v):
    return jnp.concatenate([v, jnp.zeros_like(v)], axis=0).astype(BF)


def _layernorm(x):
    c = x - jnp.sum(x, axis=-1, keepdims=True) * (1.0 / D)
    v = jnp.sum(c * c, axis=-1, keepdims=True) * (1.0 / D)
    return c, jnp.broadcast_to(1.0 / jnp.sqrt(v + EPS), (8, 128))


def _w(ref, r0, c):
    return pltpu.bitcast(ref[pl.ds(r0, 8), c].reshape(64, 128), BF)


def _mm(lhs, w):
    return jnp.dot(lhs, w, preferred_element_type=F32)[0:8]


def _halves(w):
    return pltpu.bitcast(w << 16, F32), pltpu.bitcast(w & jnp.int32(-65536), F32)


def make_kernel(layers=2, extra=0, prio=0, unroll=1, cgran=5, nx=2, ne=6, nxl=13, rg=4, lag=5, tstep=2, ktie=False, sord=2,
                f0=-.02, f3=.88, ft0=-.05, ft=.36, tlag=1.0, fp=None, fl=.85, w2split=(0, 7, 12), sstore=True):
  NV = NC - nx
  NP = -(-NV // cgran)
  w2_sem = [5, 0, 1, 2]
  echunks = [int((i + 0.5) * NV / ne) for i in range(ne)]

  def kernel(x_hbm, k_hbm, v_hbm, wq_hbm, wo_hbm, w1_hbm, w3_hbm, w2_hbm, o_ref,
             ks, vs, ve, wqs, wos, w1s, w3s, w2s, xs, lq, lo_buf, lx, accs, accx, dens, masks, sems, *ps):
    *ps, x_ref = ps
    def retiled(src, dst, sem):
        d = dst.bitcast(BF)
        return [pltpu.make_async_copy(src.at[:, hf], d.at[:, :, pl.ds(8 * hf, 8), :], sem)
                for hf in range(2)]

    def kv_copy(hbm, buf, g, sem):
        return retiled(hbm.at[pl.ds(24 * g, 24), :, pl.ds(C0, NC)], buf.at[pl.ds(24 * g, 24)], sem)

    k_cp = lambda g: kv_copy(k_hbm, ks, g, sems.at[g & 1])
    v_cp = lambda g: kv_copy(v_hbm, vs, g, sems.at[2 + (g & 1)])
    wq_cp = lambda: retiled(wq_hbm, wqs.at[pl.ds(0, D // 16)], sems.at[4])
    wo_cp = lambda: [pltpu.make_async_copy(wo_hbm, wos.bitcast(BF), sems.at[5])]
    w13_cp = lambda: retiled(w1_hbm, w1s, sems.at[4]) + retiled(w3_hbm, w3s, sems.at[4])

    def w2_cp(i):
        rows = pl.ds(8 * w2split[i], 8 * (w2split[i + 1] - w2split[i]))
        return retiled(w2_hbm.at[rows], w2s.at[rows], sems.at[w2_sem[i]])

    def start(cps):
        for i, c in enumerate(cps):
            c.start(priority=(i % 2) * prio)

    def wait(cps):
        for c in cps:
            c.wait()

    x_cp = pltpu.make_async_copy(x_hbm, x_ref, sems.at[3])
    start(wq_cp()); x_cp.start(); start(k_cp(0)); start(wo_cp())

    sub = lax.broadcasted_iota(I32, (8, 128), 0)
    lane = lax.broadcasted_iota(I32, (8, 128), 1)
    for t in range(3):
        for j in range(4):
            masks[3 * j + t] = jnp.where(sub == j, jnp.where(128 * t + lane >= DH, -65536, 65535), 0)
    x_cp.wait()

    LQ, LX, LS, LJ, LP, LO = 0, 12, 17, 18, 42, 44
    unit = [None, True]

    def tie(v, lag=lag):
        if unit[0] is not None and unit[1]:
            ps[(unit[0] + lag) % NP][2 * cgran] = v

    def put(buf, i, v):
        buf[i] = pltpu.bitcast(v, I32)

    def get(buf, i, g, dtype=BF):
        return pltpu.bitcast(buf[i + 4 * (g >> 8)], dtype)

    def stage_q(g, out):
        for kk in range(ND):
            for t in range(3):
                y = _mm(get(lq, LX + kk, g), _w(wqs, 8 * kk, 3 * g + t))
                if kk == 0:
                    out.append(y)
                else:
                    out[t] = out[t] + y
                tie(out[t])
                yield

    def store_q(qs):
        for t, q in enumerate(qs):
            q = pltpu.bitcast(_rows16(q * pltpu.bitcast(lq[LS], F32)), I32)
            for j in range(4):
                lq[LQ + 3 * j + t] = q & masks[3 * j + t]

    def both_halves(op, v):
        v = op(v, pltpu.roll(v, 2, 0))
        return op(v, pltpu.roll(v, 4, 0))

    def stage_s(g, s):
        s.extend([None] * (NC // 4))
        if sord == 1:
            order = [(2 * j1 + j0, t, m) for m in range(NC // 4) for j1 in range(2) for t in range(3) for j0 in range(2)]
        elif sord == 0:
            order = [(j, t, m) for j in range(4) for t in range(3) for m in range(NC // 4)]
        elif sord == 4:
            order = [(j, t, m0 + m) for m0 in (0, 4) for t in range(3) for j in range(4) for m in range(4)]
        elif sord == 2:
            order = [(j, t, m) for m in range(NC // 4) for t in range(3) for j in range(4)]
        else:
            order = [(j, t, m + mm) for m in range(0, NC // 4, 2) for t in range(3) for j in range(4) for mm in range(2)]
        for j, t, m in order:
            y = _mm(get(lq, LQ + 3 * j + t, g), _w(ks, 24 * g + 8 * t, 4 * m + j))
            s[m] = y if s[m] is None else s[m] + y
            tie(s[m])
            yield

    def stage_p(s, g):
        mx = functools.reduce(jnp.maximum, s)
        mx = jnp.max(both_halves(jnp.maximum, mx), axis=-1, keepdims=True)
        e = [jnp.exp((v - mx) * SCALE) for v in s]
        for c in range(NC):
            m, j = divmod(c, 4)
            if c >= NV:
                put(lx, LP + c - NV, _rows8(jnp.where(sub // 2 == j, e[m], 0.0)))
                continue
            for hh in range(2):
                ps[c // cgran][2 * (c % cgran) + hh] = jnp.broadcast_to(e[m][2 * j + hh:2 * j + hh + 1], (8, 128))
        dens[g & 3] = both_halves(jnp.add, functools.reduce(jnp.add, e))

    def retile_wo():
        def body(r, _):
            v = [wos[r, c] for c in range(ND)]
            u = [pltpu.roll(a, 4, 0) for a in v]
            for c, (a, b) in enumerate(((v[0], v[2]), (u[0], u[3]), (v[1], v[3]), (u[1], u[4]), (v[2], v[4]))):
                wos[r, c] = jnp.where(sub < 4, a, b)
        lax.fori_loop(0, NT, body, None, unroll=2)

    def expand(g, xc):
        def flip(t, _):
            for c in xc:
                w = _w(vs, 24 * g + 8 * t, c).T
                vs[pl.ds(24 * g + 8 * t, 8), c] = pltpu.bitcast(w, I32).reshape(8, 8, 128)
        lax.fori_loop(0, 3, flip, None)

        def body(r, _):
            for i, c in enumerate(echunks):
                lo, hi = _halves(vs[24 * g + r, c])
                vs[24 * g + r, c] = pltpu.bitcast(lo, I32)
                ve[24 * g + r, i] = hi
        if ne:
            lax.fori_loop(0, 24, body, None)

    def stage_v(g, chunks, switch):
        for hh in range(2):
            for r0 in range(0, 12, rg):
                acc = [None] * (2 * rg)
                for c in chunks:
                    p = ps[c // cgran][2 * (c % cgran) + hh + 4 * (g >> 8)]
                    for r in range(rg):
                        row = 24 * g + 12 * hh + r0 + r
                        if c in echunks:
                            parts = pltpu.bitcast(vs[row, c], F32), ve[row, echunks.index(c)]
                        else:
                            parts = _halves(vs[row, c])
                        for i in range(2):
                            a = parts[i] * p
                            acc[rg * i + r] = a if c == chunks[0] else acc[rg * i + r] + a
                    if c % cgran == cgran - 1 or c == chunks[-1]:
                        for bufs in switch():
                            if bufs[1] is None:
                                for i, v in enumerate(acc[::tstep]):
                                    put(bufs[0], LJ + i, v)
                            else:
                                bufs[0][bufs[1], 0] = pltpu.bitcast(acc[-1], I32)
                        unit[0] += 1
                        yield
                for r in range(rg):
                    for i in range(2):
                        accs[pl.ds(DH * hh + 16 * (r0 + r) + i, 8, stride=2), :] = acc[rg * i + r]

    def stage_x(g, chunks):
        acc = [jnp.zeros((8, 128), F32)] * 3
        for n, c in enumerate(chunks):
            for t in range(3):
                y = _mm(get(lx, LP + c - NV + (NC if c < NV else 0), g), _w(vs, 24 * g + 8 * t, c))
                acc[t] = y if n == 0 else acc[t] + y
                tie(acc[t])
                yield
        for t in range(3 if chunks else 0):
            accx[t] = jnp.where((sub & 1) == (128 * t + lane >= DH).astype(I32), acc[t], 0.0)

    def stage_t(g, with_x):
        inv = 1.0 / jnp.sum(dens[g & 3], axis=-1, keepdims=True)
        inv0 = jnp.broadcast_to(inv[0:1], (8, 128))
        inv1 = jnp.broadcast_to(inv[1:2], (8, 128))
        for t in range(3):
            blk = accs[pl.ds(pl.multiple_of(128 * t + 128 * (g >> 8), 128), 128), :]
            o = jnp.sum(blk.T.reshape(16, 8, 128), axis=0)
            if with_x:
                o = o + accx[t]
            o = jnp.broadcast_to(jnp.sum(o, axis=0, keepdims=True), (8, 128))
            o = o * (inv0, jnp.where(lane >= DH - 128, inv1, inv0), inv1)[t]
            put(lo_buf, LO + t, _rows16(o))
            tie(o, min(NP - 1, int(tlag * NP)))
            yield

    def stage_o(g):
        acc = [xs[c + 8 * (g >> 8)] for c in range(ND)]
        for t in range(3):
            for c in range(ND):
                acc[c] = acc[c] + _mm(get(lo_buf, LO + t, g), _w(wos, 24 * g + 8 * t, c))
                tie(acc[c])
                yield
        for c in range(ND):
            xs[c] = acc[c]

    def run(*gens):
        for gen in gens:
            for _ in gen:
                pass

    def mix(mxu, side, g, chunks, f0=f0, f3=f3, back=True):
        nv = 2 * (12 // rg) * len({c // cgran for c in chunks})
        tot = sum(n * cost for _, n, cost, _, _ in mxu)
        ev, gens, pos = [], [], 0
        for gen, n, cost, lbuf, wbuf in mxu:
            for k in range(n):
                ev.append((f0 + (f3 - f0) * (pos + 0.5 * cost) / tot, len(gens), lbuf, wbuf))
                pos += cost
            ev.append((f0 + (f3 - f0) * pos / tot - 1e-9, len(gens), None, None))
            gens.append(gen)
        for gen, n, t0, t1 in side:
            ev += [(t0 + (t1 - t0) * (k + 0.5) / n, len(gens), None, None) for k in range(n)]
            gens.append(gen)
        ev += [((k + 0.5) / nv, len(gens), None, None) for k in range(nv)] + [(2, len(gens), None, None)]
        ev.sort(key=lambda e: e[:2])
        now = [0]

        def switch():
            out = {}
            for e in ev[now[0] + 1:]:
                if e[1] == len(gens) - 1:
                    break
                if e[2] is not None:
                    out[id(e[2])] = (e[2], None)
                if e[3] is not None and ktie:
                    out[id(e[3][0])] = e[3]
            return list(out.values())

        gens.append(stage_v(g, chunks, switch))
        unit[:] = 0, back
        for now[0], e in enumerate(ev):
            next(gens[e[1]], None)
        unit[0] = None

    def get_x():
        return jnp.concatenate([xs[c] for c in range(ND)], axis=1)

    v_chunks, x_chunks = list(range(NV)), list(range(NV, NC))
    moved = [c for c in reversed(v_chunks) if c not in echunks][:nxl]

    def attend(g, with_o):
        s, q = [], []
        mxu = [(stage_s(g + 1, s), 96, 1, lq, (ks, NT)), (stage_x(g, x_chunks), 3 * nx, 1, lx, None),
               (stage_q(jnp.minimum(g + 2, NG - 1), q), 15, 1, lq, (wqs, D // 16))]
        side = []
        if with_o:
            mxu.append((stage_o(g - 1), 15, 1, lo_buf, None))
            side.append((stage_t(g - 1, nx > 0), 3, ft0, ft))
        mix(mxu, side, g, v_chunks)
        store_q(q)
        stage_p(s, g + 1)

    def layer(l, _):
        on_first = pl.when(l == 0)
        z = l >> 8

        @on_first
        def _():
            wait(wq_cp())
            start(k_cp(1)); start(v_cp(0))
            wait(k_cp(0))
            start(k_cp(2)); start(v_cp(1))
        xc, rstd = _layernorm(get_x())
        xc = _rows16(xc)
        for kk in range(ND):
            put(lq, LX + kk, xc[:, 128 * kk:128 * (kk + 1)])
        put(lq, LS, rstd)
        s, q = [], []
        run(stage_q(z, q))
        store_q(q)
        q = []
        run(stage_s(z, s), stage_q(z + 1, q))
        stage_p(s, 0)
        store_q(q)

        @on_first
        def _():
            wait(wo_cp()); wait(k_cp(1)); wait(v_cp(0))
            start(k_cp(3)); start(v_cp(2))
            expand(0, x_chunks)
            retile_wo()
        attend(z, False)

        def fetch(g):
            wait(k_cp(g + 1)); wait(v_cp(g))

            @pl.when(g + 3 < NG)
            def _():
                start(k_cp(g + 3))

            @pl.when(g + 2 < NG)
            def _():
                start(v_cp(g + 2))

            @pl.when(g + 3 == NG)
            def _():
                start(w13_cp())

            @pl.when(g + 2 == NG)
            def _():
                start(w2_cp(0))
            expand(g, x_chunks)

        def step(i, _):
            i = jnp.minimum(i, (NG - 2) // unroll - 1) if extra else i
            g = 1 + unroll * i
            on_first(lambda: lax.fori_loop(g, g + unroll, lambda g, _: fetch(g), None))
            for u in range(unroll):
                attend(g + u, True)

        lax.fori_loop(0, (NG - 2) // unroll + (extra * l if extra else 0), step, None)

        @on_first
        def _():
            wait(v_cp(NG - 1))
            for i in range(1, len(w2split) - 1):
                start(w2_cp(i))
            expand(NG - 1, x_chunks + moved)
            wait(w13_cp())
        for c in moved:
            p0, p1 = (ps[c // cgran][2 * (c % cgran) + hh] for hh in range(2))
            put(lx, LP + c - NV + NC, _rows8(jnp.where(sub == 0, p0, jnp.where(sub == 1, p1, 0.0))))
        t = stage_t(z + NG - 2, nx > 0)
        mix([(stage_x(z + NG - 1, x_chunks + moved), 3 * (nx + nxl), 1, lx, None),
             (stage_o(z + NG - 2), 15, 1, lo_buf, None)],
            [(t, 3, ft0, ft)], z + NG - 1, [c for c in v_chunks if c not in moved], f3=fl, back=False)
        run(stage_t(z + NG - 1, nx + nxl > 0), stage_o(z + NG - 1))

        on_first(lambda: wait(w2_cp(0)))
        x = get_x()
        xc, rstd = _layernorm(x)
        xc = _rows16(xc)
        hs = []
        for c in range(F // 128):
            gate, up = (rstd * functools.reduce(jnp.add, [
                _mm(xc[:, 128 * kk:128 * (kk + 1)], _w(w, 8 * kk, c)) for kk in range(ND)]) for w in (w1s, w3s))
            hs.append(_rows16(gate * (1.0 / (1.0 + jnp.exp(-gate))) * up))
        acc = [x[:, 128 * c:128 * (c + 1)] for c in range(ND)]
        for i in range(len(w2split) - 1):
            if i:
                on_first(lambda: wait(w2_cp(i)))
            for kk in range(w2split[i], w2split[i + 1]):
                for c in range(ND):
                    acc[c] = acc[c] + _mm(hs[kk], _w(w2s, 8 * kk, c))
        for c in range(ND):
            xs[c] = acc[c]

    x = jnp.broadcast_to(x_ref[0].astype(F32), (8, D))
    for c in range(ND):
        xs[c] = x[:, 128 * c:128 * (c + 1)]
    lax.fori_loop(0, layers, layer, None)
    o_ref[0] = get_x()[0:1].astype(o_ref.dtype)

  def tiles(r, c, pad=0):
      return pltpu.VMEM((r // 16 + pad, c // 128, 8, 128), I32)

  def vregs(n, dtype):
      return pltpu.VMEM((-(-n // 4) * 4, 8, 128), dtype)

  scratch = [
      tiles(H * DH, W, int(ktie)), tiles(H * DH, W), pltpu.VMEM((NT, max(ne, 1), 8, 128), F32),
      tiles(D, H * DH, int(ktie)), tiles(H * DH, D), tiles(D, F), tiles(D, F), tiles(F, D),
      vregs(8, F32), vregs(44, I32), vregs(48, I32), vregs(44 + NC, I32),
      pltpu.VMEM((2 * DH, 128), F32), vregs(4, F32), vregs(4, F32), vregs(12, I32),
      pltpu.SemaphoreType.DMA((6,)),
  ] + [vregs(2 * cgran + 1, F32)] * NP + [pltpu.VMEM((1, 1, D), BF)]
  return kernel, scratch


def build(flags=None, **kw):
  def f(A_x, A_k_cache, A_v_cache, A_wq, A_wo, B_x, B_w1, B_w3, B_w2):
    def cache_view(c):
        return c.transpose(0, 1, 3, 2).reshape(NT, 2, 8, SK // 128, 128).transpose(0, 1, 3, 2, 4)

    def weight_view(w):
        return w.reshape(w.shape[0] // 16, 2, 8, w.shape[1] // 128, 128).transpose(0, 1, 3, 2, 4)

    kernel, scratch = make_kernel(**kw)
    return pl.pallas_call(
        kernel,
        out_shape=jax.ShapeDtypeStruct(A_x.shape, A_x.dtype),
        in_specs=[pl.BlockSpec(memory_space=pl.ANY)] * 8,
        out_specs=pl.BlockSpec(memory_space=pltpu.VMEM),
        scratch_shapes=scratch,
        compiler_params=pltpu.CompilerParams(vmem_limit_bytes=128 * 2**20, flags=flags),
        name="fused",
    )(A_x, cache_view(A_k_cache), cache_view(A_v_cache),
      weight_view(A_wq), weight_view(A_wo).reshape(NT, ND, 16, 128), *[weight_view(w) for w in (B_w1, B_w3, B_w2)])
  return f


@jax.jit
def pallas_interleave_layers__sliding_block_cached__glu_gated_swiglu__decode_kernel(
    A_x: jax.Array,
    A_k_cache: jax.Array,
    A_v_cache: jax.Array,
    A_wq: jax.Array,
    A_wo: jax.Array,
    B_x: jax.Array,
    B_w1: jax.Array,
    B_w3: jax.Array,
    B_w2: jax.Array,
):
    return build()(A_x, A_k_cache, A_v_cache, A_wq, A_wo, B_x, B_w1, B_w3, B_w2)
```

```python
import functools

import jax
import jax.numpy as jnp
from jax import lax
from jax.experimental import pallas as pl
from jax.experimental.pallas import tpu as pltpu

D, H, DH, SK, F = 640, 32, 192, 32768, 1536
WINDOW = min(4096, max(256, SK // 4))
NC = WINDOW // 128
C0 = (SK - WINDOW) // 128
NG = H // 2
NT = H * DH // 16
ND = D // 128
RG = 4
BF, F32, I32 = jnp.bfloat16, jnp.float32, jnp.int32
SCALE = DH ** -0.5
EPS = 1e-5


def _rows16(v):
    return jnp.concatenate([v, v], axis=0).astype(BF)


def _rows8(v):
    return jnp.concatenate([v, jnp.zeros_like(v)], axis=0).astype(BF)


def _layernorm(x):
    c = x - jnp.sum(x, axis=-1, keepdims=True) * (1.0 / D)
    v = jnp.sum(c * c, axis=-1, keepdims=True) * (1.0 / D)
    return c, jnp.broadcast_to(1.0 / jnp.sqrt(v + EPS), (8, 128))


def _tile(ref, r0, c):
    return pltpu.bitcast(ref[pl.ds(r0, 8), c].reshape(64, 128), BF)


def _mm(lhs, w):
    return jnp.dot(lhs, w, preferred_element_type=F32)[0:8]


def _halves(w):
    return pltpu.bitcast(w << 16, F32), pltpu.bitcast(w & jnp.int32(-65536), F32)


def _over_chunks(op, v):
    v = op(v, pltpu.roll(v, 2, 0))
    return op(v, pltpu.roll(v, 4, 0))


def make_kernel(nx=3, ne=6, cgran=4, lag=7, f0=.02, f1=.86, ft0=-.05, ft1=.46, w2_split=7):
    nvc = NC - nx
    n_pbuf = -(-nvc // cgran)
    v_chunks, x_chunks = list(range(nvc)), list(range(nvc, NC))
    e_chunks = [int((i + 0.5) * nvc / ne) for i in range(ne)]
    w2_parts = ((0, w2_split), (w2_split, F // 128))
    LANE0 = 4
    L_Q, L_X, L_RSTD = LANE0, LANE0 + 12, LANE0 + 12 + ND

    def kernel(x_hbm, k_hbm, v_hbm, wq_hbm, wo_hbm, w1_hbm, w3_hbm, w2_hbm, o_ref,
               ks, vs, ve, wqs, wos, w1s, w3s, w2s, xs, lq, lo, lp, accs, accx, dens, masks, sems, *rest):
        *ps, x_ref = rest

        def retiled(src, dst, sem):
            dst = dst.bitcast(BF)
            return [pltpu.make_async_copy(src.at[:, i], dst.at[:, :, pl.ds(8 * i, 8), :], sems.at[sem])
                    for i in range(2)]

        def cache_cp(hbm, buf, g, sem):
            return retiled(hbm.at[pl.ds(24 * g, 24), :, pl.ds(C0, NC)], buf.at[pl.ds(24 * g, 24)], sem)

        def w2_cp(i):
            rows = pl.ds(8 * w2_parts[i][0], 8 * (w2_parts[i][1] - w2_parts[i][0]))
            return retiled(w2_hbm.at[rows], w2s.at[rows], (5, 0)[i])

        k_cp = lambda g: cache_cp(k_hbm, ks, g, g & 1)
        v_cp = lambda g: cache_cp(v_hbm, vs, g, 2 + (g & 1))
        wq_cp = lambda: retiled(wq_hbm, wqs, 4)
        wo_cp = lambda: [pltpu.make_async_copy(wo_hbm, wos.bitcast(BF), sems.at[5])]
        w13_cp = lambda: retiled(w1_hbm, w1s, 4) + retiled(w3_hbm, w3s, 4)

        def start(cps):
            for c in cps:
                c.start()

        def wait(cps):
            for c in cps:
                c.wait()

        x_cp = pltpu.make_async_copy(x_hbm, x_ref, sems.at[3])
        start(wq_cp())
        x_cp.start()
        start(k_cp(0))
        start(wo_cp())

        sub = lax.broadcasted_iota(I32, (8, 128), 0)
        lane = lax.broadcasted_iota(I32, (8, 128), 1)
        head = [(128 * t + lane >= DH).astype(I32) for t in range(3)]
        for t in range(3):
            for j in range(4):
                masks[3 * j + t] = jnp.where(sub == j, jnp.where(head[t] == 1, -65536, 65535), 0)
        x_cp.wait()

        def retile_wo():
            def body(r, _):
                v = [wos[r, c] for c in range(ND)]
                u = [pltpu.roll(a, 4, 0) for a in v]
                pairs = ((v[0], v[2]), (u[0], u[3]), (v[1], v[3]), (u[1], u[4]), (v[2], v[4]))
                for c, (a, b) in enumerate(pairs):
                    wos[r, c] = jnp.where(sub < 4, a, b)
            lax.fori_loop(0, NT, body, None, unroll=2)

        def prepare_v(g, mxu_chunks, f32_chunks):
            def flip(t, _):
                for c in mxu_chunks:
                    w = _tile(vs, 24 * g + 8 * t, c).T
                    vs[pl.ds(24 * g + 8 * t, 8), c] = pltpu.bitcast(w, I32).reshape(8, 8, 128)

            def unpack(r, _):
                for i, c in enumerate(f32_chunks):
                    even, odd = _halves(vs[24 * g + r, c])
                    vs[24 * g + r, c] = pltpu.bitcast(even, I32)
                    ve[24 * g + r, i] = odd
            lax.fori_loop(0, 3, flip, None)
            if f32_chunks:
                lax.fori_loop(0, 24, unpack, None)

        unit = [None]

        def tie(v, lag=lag):
            if unit[0] is not None:
                ps[(unit[0] + lag) % n_pbuf][2 * cgran] = v

        def put(buf, i, v):
            buf[i] = pltpu.bitcast(v, I32)

        def get(buf, i, g):
            return pltpu.bitcast(buf[i + 4 * (g >> 8)], BF)

        def project_q(g, q):
            q.extend([None] * 3)
            for kk in range(ND):
                for t in range(3):
                    y = _mm(get(lq, L_X + kk, g), _tile(wqs, 8 * kk, 3 * g + t))
                    q[t] = y if kk == 0 else q[t] + y
                    tie(q[t])
                    yield

        def store_q(q):
            for t in range(3):
                packed = pltpu.bitcast(_rows16(q[t] * pltpu.bitcast(lq[L_RSTD], F32)), I32)
                for j in range(4):
                    lq[L_Q + 3 * j + t] = packed & masks[3 * j + t]

        def scores(g, s):
            for m in range(NC // 4):
                acc = None
                for t in range(3):
                    for j in range(4):
                        y = _mm(get(lq, L_Q + 3 * j + t, g), _tile(ks, 24 * g + 8 * t, 4 * m + j))
                        acc = y if acc is None else acc + y
                        tie(acc)
                        yield
                s.append(acc)

        def softmax(s, g):
            top = jnp.max(_over_chunks(jnp.maximum, functools.reduce(jnp.maximum, s)), axis=-1, keepdims=True)
            e = [jnp.exp((v - top) * SCALE) for v in s]
            for c in range(NC):
                m, j = divmod(c, 4)
                if c in x_chunks:
                    put(lp, LANE0 + c - nvc, _rows8(jnp.where(sub // 2 == j, e[m], 0.0)))
                    continue
                for h in range(2):
                    ps[c // cgran][2 * (c % cgran) + h] = jnp.broadcast_to(e[m][2 * j + h:2 * j + h + 1], (8, 128))
            dens[g & 3] = _over_chunks(jnp.add, functools.reduce(jnp.add, e))

        def values_vpu(g, next_lhs):
            for h in range(2):
                for r0 in range(0, 12, RG):
                    acc = [None] * (2 * RG)
                    for c in v_chunks:
                        p = ps[c // cgran][2 * (c % cgran) + h + 4 * (g >> 8)]
                        for r in range(RG):
                            row = 24 * g + 12 * h + r0 + r
                            if c in e_chunks:
                                parts = pltpu.bitcast(vs[row, c], F32), ve[row, e_chunks.index(c)]
                            else:
                                parts = _halves(vs[row, c])
                            for i in range(2):
                                a = parts[i] * p
                                acc[RG * i + r] = a if c == 0 else acc[RG * i + r] + a
                        if c % cgran == cgran - 1 or c == nvc - 1:
                            for buf in next_lhs():
                                for i, v in enumerate(acc[::2]):
                                    put(buf, i, v)
                            unit[0] += 1
                            yield
                    for r in range(RG):
                        for i in range(2):
                            accs[pl.ds(DH * h + 16 * (r0 + r) + i, 8, stride=2), :] = acc[RG * i + r]

        def values_mxu(g, chunks):
            acc = [None] * 3
            for c in chunks:
                if c in x_chunks:
                    p = lambda: get(lp, LANE0 + c - nvc, g)
                else:
                    p0, p1 = (ps[c // cgran][2 * (c % cgran) + h] for h in range(2))
                    p01 = _rows8(jnp.where(sub == 0, p0, jnp.where(sub == 1, p1, 0.0)))
                    p = lambda: p01
                for t in range(3):
                    y = _mm(p(), _tile(vs, 24 * g + 8 * t, c))
                    acc[t] = y if acc[t] is None else acc[t] + y
                    tie(acc[t])
                    yield
            for t in range(3):
                accx[t] = jnp.where((sub & 1) == head[t], acc[t], 0.0)

        def finish_values(g, with_vpu=True):
            inv = 1.0 / jnp.sum(dens[g & 3], axis=-1, keepdims=True)
            inv0 = jnp.broadcast_to(inv[0:1], (8, 128))
            inv1 = jnp.broadcast_to(inv[1:2], (8, 128))
            for t in range(3):
                o = accx[t]
                if with_vpu:
                    blk = accs[pl.ds(pl.multiple_of(128 * t + 128 * (g >> 8), 128), 128), :]
                    o = o + jnp.sum(blk.T.reshape(16, 8, 128), axis=0)
                o = jnp.broadcast_to(jnp.sum(o, axis=0, keepdims=True), (8, 128))
                o = o * (inv0, jnp.where(head[1] == 1, inv1, inv0), inv1)[t]
                put(lo, LANE0 + t, _rows16(o))
                tie(o, n_pbuf - 1)
                yield

        def project_o(g):
            acc = [xs[c + 8 * (g >> 8)] for c in range(ND)]
            for t in range(3):
                for c in range(ND):
                    acc[c] = acc[c] + _mm(get(lo, LANE0 + t, g), _tile(wos, 24 * g + 8 * t, c))
                    tie(acc[c])
                    yield
            for c in range(ND):
                xs[c] = acc[c]

        def run(*gens):
            for gen in gens:
                for _ in gen:
                    pass

        def attend(g, with_o):
            s, q = [], []
            mxu = [(scores(g + 1, s), 3 * NC, lq), (values_mxu(g, x_chunks), 3 * nx, lp),
                   (project_q(jnp.minimum(g + 2, NG - 1), q), 3 * ND, lq)]
            if with_o:
                mxu.append((project_o(g - 1), 3 * ND, lo))
            step = (f1 - f0) / sum(n for _, n, _ in mxu)
            events, gens, pos = [], [], 0
            for gen, n, buf in mxu:
                events += [(f0 + step * (pos + k + 0.5), len(gens), buf) for k in range(n)]
                pos += n
                events.append((f0 + step * pos, len(gens), None))
                gens.append(gen)
            if with_o:
                events += [(ft0 + (ft1 - ft0) * (k + 0.5) / 3, len(gens), None) for k in range(3)]
                gens.append(finish_values(g - 1))
            n_units = 2 * (12 // RG) * n_pbuf
            events += [((k + 0.5) / n_units, len(gens), None) for k in range(n_units)] + [(2, len(gens), None)]
            events.sort(key=lambda ev: ev[:2])
            now = [0]

            def next_lhs():
                bufs = []
                for _, i, buf in events[now[0] + 1:]:
                    if i == len(gens) - 1:
                        break
                    if buf is not None and not any(buf is b for b in bufs):
                        bufs.append(buf)
                return bufs

            gens.append(values_vpu(g, next_lhs))
            unit[0] = 0
            for now[0], ev in enumerate(events):
                next(gens[ev[1]], None)
            unit[0] = None
            store_q(q)
            softmax(s, g + 1)

        def load_x():
            return jnp.concatenate([xs[c] for c in range(ND)], axis=1)

        def layer(l, _):
            first = pl.when(l == 0)
            z = l >> 8

            @first
            def _():
                wait(wq_cp())
                start(k_cp(1))
                start(v_cp(0))
                wait(k_cp(0))
                start(k_cp(2))
                start(v_cp(1))
            xc, rstd = _layernorm(load_x())
            xc = _rows16(xc)
            for kk in range(ND):
                put(lq, L_X + kk, xc[:, 128 * kk:128 * (kk + 1)])
            put(lq, L_RSTD, rstd)
            s, q0, q1 = [], [], []
            run(project_q(z, q0))
            store_q(q0)
            run(scores(z, s), project_q(z + 1, q1))
            softmax(s, 0)
            store_q(q1)

            @first
            def _():
                wait(wo_cp())
                wait(k_cp(1))
                wait(v_cp(0))
                start(k_cp(3))
                start(v_cp(2))
                prepare_v(0, x_chunks, e_chunks)
                retile_wo()
            attend(z, False)

            def pair(g, _):
                @first
                def _():
                    wait(k_cp(g + 1))
                    wait(v_cp(g))
                    pl.when(g + 3 < NG)(lambda: start(k_cp(g + 3)))
                    pl.when(g + 2 < NG)(lambda: start(v_cp(g + 2)))
                    pl.when(g + 3 == NG)(lambda: start(w13_cp()))
                    pl.when(g + 2 == NG)(lambda: start(w2_cp(0)))
                    prepare_v(g, x_chunks, e_chunks)
                attend(g, True)

            lax.fori_loop(1, NG - 1, pair, None)

            @first
            def _():
                wait(v_cp(NG - 1))
                start(w2_cp(1))
                prepare_v(NG - 1, x_chunks + v_chunks, [])
                wait(w13_cp())
            run(finish_values(z + NG - 2), values_mxu(z + NG - 1, x_chunks + v_chunks), project_o(z + NG - 2),
                finish_values(z + NG - 1, False), project_o(z + NG - 1))

            first(lambda: wait(w2_cp(0)))
            x = load_x()
            xc, rstd = _layernorm(x)
            xc = _rows16(xc)
            hs = []
            for c in range(F // 128):
                gate, up = (rstd * functools.reduce(jnp.add, [
                    _mm(xc[:, 128 * kk:128 * (kk + 1)], _tile(w, 8 * kk, c)) for kk in range(ND)])
                            for w in (w1s, w3s))
                hs.append(_rows16(gate * jax.nn.sigmoid(gate) * up))
            acc = [x[:, 128 * c:128 * (c + 1)] for c in range(ND)]
            for i, part in enumerate(w2_parts):
                if i:
                    first(lambda: wait(w2_cp(i)))
                for kk in range(*part):
                    for c in range(ND):
                        acc[c] = acc[c] + _mm(hs[kk], _tile(w2s, 8 * kk, c))
            for c in range(ND):
                xs[c] = acc[c]

        x = jnp.broadcast_to(x_ref[0].astype(F32), (8, D))
        for c in range(ND):
            xs[c] = x[:, 128 * c:128 * (c + 1)]
        lax.fori_loop(0, 2, layer, None)
        o_ref[0] = load_x()[0:1].astype(o_ref.dtype)

    def tiles(r, c):
        return pltpu.VMEM((r // 16, c // 128, 8, 128), I32)

    def vregs(n, dtype):
        return pltpu.VMEM((-(-n // 4) * 4, 8, 128), dtype)

    scratch = [
        tiles(H * DH, WINDOW), tiles(H * DH, WINDOW), pltpu.VMEM((NT - 24, ne, 8, 128), F32),
        tiles(D, H * DH), tiles(H * DH, D), tiles(D, F), tiles(D, F), tiles(F, D),
        vregs(ND, F32), vregs(L_RSTD + 1, I32), vregs(LANE0 + 3, I32), vregs(LANE0 + nx, I32),
        pltpu.VMEM((2 * DH, 128), F32), vregs(3, F32), vregs(4, F32), vregs(12, I32),
        pltpu.SemaphoreType.DMA((6,)),
    ] + [vregs(2 * cgran + 1, F32)] * n_pbuf + [pltpu.VMEM((1, 1, D), BF)]
    return kernel, scratch


def build(**schedule):
    def call(A_x, A_k_cache, A_v_cache, A_wq, A_wo, B_x, B_w1, B_w3, B_w2):
        def tile_view(w):
            return w.reshape(w.shape[0] // 16, 2, 8, w.shape[1] // 128, 128).transpose(0, 1, 3, 2, 4)

        def cache_view(c):
            return tile_view(c.transpose(0, 1, 3, 2).reshape(H * DH, SK))

        kernel, scratch = make_kernel(**schedule)
        return pl.pallas_call(
            kernel,
            out_shape=jax.ShapeDtypeStruct(A_x.shape, A_x.dtype),
            in_specs=[pl.BlockSpec(memory_space=pl.ANY)] * 8,
            out_specs=pl.BlockSpec(memory_space=pltpu.VMEM),
            scratch_shapes=scratch,
            compiler_params=pltpu.CompilerParams(vmem_limit_bytes=128 * 2**20),
            name="fused",
        )(A_x, cache_view(A_k_cache), cache_view(A_v_cache), tile_view(A_wq),
          tile_view(A_wo).reshape(NT, ND, 16, 128), tile_view(B_w1), tile_view(B_w3), tile_view(B_w2))
    return call


@jax.jit
def pallas_interleave_layers__sliding_block_cached__glu_gated_swiglu__decode_kernel(
    A_x: jax.Array,
    A_k_cache: jax.Array,
    A_v_cache: jax.Array,
    A_wq: jax.Array,
    A_wo: jax.Array,
    B_x: jax.Array,
    B_w1: jax.Array,
    B_w3: jax.Array,
    B_w2: jax.Array,
):
    return build(ne=7, nx=2, cgran=3, lag=9, f0=-.02, f1=.9, ft0=0)(A_x, A_k_cache, A_v_cache, A_wq, A_wo, B_x, B_w1, B_w3, B_w2)
```

```python
import functools

import jax
import jax.numpy as jnp
from jax import lax
from jax.experimental import pallas as pl
from jax.experimental.pallas import tpu as pltpu

D, H, DH, SK, F = 640, 32, 192, 32768, 1536
WINDOW = min(4096, max(256, SK // 4))
NC = WINDOW // 128
C0 = (SK - WINDOW) // 128
NG = H // 2
NT = H * DH // 16
ND = D // 128
RG = 4
BF, F32, I32 = jnp.bfloat16, jnp.float32, jnp.int32
SCALE = DH ** -0.5
EPS = 1e-5


def _rows16(v):
    return jnp.concatenate([v, v], axis=0).astype(BF)


def _rows8(v):
    return jnp.concatenate([v, jnp.zeros_like(v)], axis=0).astype(BF)


def _layernorm(x):
    c = x - jnp.sum(x, axis=-1, keepdims=True) * (1.0 / D)
    v = jnp.sum(c * c, axis=-1, keepdims=True) * (1.0 / D)
    return c, jnp.broadcast_to(1.0 / jnp.sqrt(v + EPS), (8, 128))


def _tile(ref, r0, c):
    return pltpu.bitcast(ref[pl.ds(r0, 8), c].reshape(64, 128), BF)


def _mm(lhs, w):
    return jnp.dot(lhs, w, preferred_element_type=F32)[0:8]


def _halves(w):
    return pltpu.bitcast(w << 16, F32), pltpu.bitcast(w & -65536, F32)


def _over_chunks(op, v):
    v = op(v, pltpu.roll(v, 2, 0))
    return op(v, pltpu.roll(v, 4, 0))


def make_kernel(nx=2, ne=7, cgran=3, lag=9, f0=.02, f1=.92, ft0=0.0, ft1=.42, w2_split=6):
    nvc = NC - nx
    n_pbuf = -(-nvc // cgran)
    v_chunks, x_chunks = list(range(nvc)), list(range(nvc, NC))
    e_chunks = [i * nvc // ne for i in range(ne)]
    w2_parts = ((0, w2_split), (w2_split, F // 128))
    L_0 = 4
    L_Q, L_X, L_RSTD = L_0, L_0 + 12, L_0 + 12 + ND

    def kernel(x_hbm, k_hbm, v_hbm, wq_hbm, wo_hbm, w1_hbm, w3_hbm, w2_hbm, o_ref,
               ks, vs, ve, wqs, wos, w1s, w3s, w2s, xs, lq, lo, lp, accs, accx, dens, masks, sems, *rest):
        *ps, x_ref = rest

        def retiled(src, dst, sem):
            dst = dst.bitcast(BF)
            return [pltpu.make_async_copy(src.at[:, i], dst.at[:, :, pl.ds(8 * i, 8), :], sems.at[sem])
                    for i in range(2)]

        def cache_cp(hbm, buf, g, sem):
            return retiled(hbm.at[pl.ds(24 * g, 24), :, pl.ds(C0, NC)], buf.at[pl.ds(24 * g, 24)], sem)

        def w2_cp(i):
            rows = pl.ds(8 * w2_parts[i][0], 8 * (w2_parts[i][1] - w2_parts[i][0]))
            return retiled(w2_hbm.at[rows], w2s.at[rows], (5, 0)[i])

        k_cp = lambda g: cache_cp(k_hbm, ks, g, g & 1)
        v_cp = lambda g: cache_cp(v_hbm, vs, g, 2 + (g & 1))
        wq_cp = lambda: retiled(wq_hbm, wqs, 4)
        wo_cp = lambda: [pltpu.make_async_copy(wo_hbm, wos.bitcast(BF), sems.at[5])]
        w13_cp = lambda: retiled(w1_hbm, w1s, 4) + retiled(w3_hbm, w3s, 4)

        def start(cps):
            for c in cps:
                c.start()

        def wait(cps):
            for c in cps:
                c.wait()

        x_cp = pltpu.make_async_copy(x_hbm, x_ref, sems.at[3])
        start(wq_cp())
        x_cp.start()
        start(k_cp(0))
        start(wo_cp())

        sub = lax.broadcasted_iota(I32, (8, 128), 0)
        lane = lax.broadcasted_iota(I32, (8, 128), 1)
        head = [(128 * t + lane >= DH).astype(I32) for t in range(3)]
        for t in range(3):
            for j in range(4):
                masks[3 * j + t] = jnp.where(sub == j, jnp.where(head[t] == 1, -65536, 65535), 0)
        x_cp.wait()

        def retile_wo():
            def body(r, _):
                v = [wos[r, c] for c in range(ND)]
                u = [pltpu.roll(a, 4, 0) for a in v]
                pairs = ((v[0], v[2]), (u[0], u[3]), (v[1], v[3]), (u[1], u[4]), (v[2], v[4]))
                for c, (a, b) in enumerate(pairs):
                    wos[r, c] = jnp.where(sub < 4, a, b)
            lax.fori_loop(0, NT, body, None, unroll=2)

        def prepare_v(g, mxu_chunks, f32_chunks):
            def flip(t, _):
                for c in mxu_chunks:
                    w = _tile(vs, 24 * g + 8 * t, c).T
                    vs[pl.ds(24 * g + 8 * t, 8), c] = pltpu.bitcast(w, I32).reshape(8, 8, 128)

            def unpack(r, _):
                for i, c in enumerate(f32_chunks):
                    even, odd = _halves(vs[24 * g + r, c])
                    vs[24 * g + r, c] = pltpu.bitcast(even, I32)
                    ve[24 * g + r, i] = odd
            lax.fori_loop(0, 3, flip, None)
            if f32_chunks:
                lax.fori_loop(0, 24, unpack, None)

        unit = [None]

        def tie(v, lag=lag):
            if unit[0] is not None:
                ps[(unit[0] + lag) % n_pbuf][2 * cgran] = v

        def put(buf, i, v):
            buf[i] = pltpu.bitcast(v, I32)

        def get(buf, i, g):
            return pltpu.bitcast(buf[i + 4 * (g >> 8)], BF)

        def project_q(g, q):
            q.extend([None] * 3)
            for kk in range(ND):
                for t in range(3):
                    y = _mm(get(lq, L_X + kk, g), _tile(wqs, 8 * kk, 3 * g + t))
                    q[t] = y if kk == 0 else q[t] + y
                    tie(q[t])
                    yield

        def store_q(q):
            for t in range(3):
                packed = pltpu.bitcast(_rows16(q[t] * pltpu.bitcast(lq[L_RSTD], F32)), I32)
                for j in range(4):
                    lq[L_Q + 3 * j + t] = packed & masks[3 * j + t]

        def scores(g, s):
            for m in range(NC // 4):
                acc = None
                for t in range(3):
                    for j in range(4):
                        y = _mm(get(lq, L_Q + 3 * j + t, g), _tile(ks, 24 * g + 8 * t, 4 * m + j))
                        acc = y if acc is None else acc + y
                        tie(acc)
                        yield
                s.append(acc)

        def softmax(s, g):
            top = jnp.max(_over_chunks(jnp.maximum, functools.reduce(jnp.maximum, s)), axis=-1, keepdims=True)
            e = [jnp.exp((v - top) * SCALE) for v in s]
            for c in range(NC):
                m, j = divmod(c, 4)
                if c in x_chunks:
                    put(lp, L_0 + c - nvc, _rows8(jnp.where(sub // 2 == j, e[m], 0.0)))
                    continue
                for h in range(2):
                    ps[c // cgran][2 * (c % cgran) + h] = jnp.broadcast_to(e[m][2 * j + h:2 * j + h + 1], (8, 128))
            dens[g & 3] = _over_chunks(jnp.add, functools.reduce(jnp.add, e))

        def values_vpu(g, next_lhs):
            for h in range(2):
                for r0 in range(0, 12, RG):
                    acc = [None] * (2 * RG)
                    for c in v_chunks:
                        p = ps[c // cgran][2 * (c % cgran) + h + 4 * (g >> 8)]
                        for r in range(RG):
                            row = 24 * g + 12 * h + r0 + r
                            if c in e_chunks:
                                parts = pltpu.bitcast(vs[row, c], F32), ve[row, e_chunks.index(c)]
                            else:
                                parts = _halves(vs[row, c])
                            for i in range(2):
                                a = parts[i] * p
                                acc[RG * i + r] = a if c == 0 else acc[RG * i + r] + a
                        if c % cgran == cgran - 1 or c == nvc - 1:
                            for buf in next_lhs():
                                for i, v in enumerate(acc[::2]):
                                    put(buf, i, v)
                            unit[0] += 1
                            yield
                    for r in range(RG):
                        for i in range(2):
                            accs[pl.ds(DH * h + 16 * (r0 + r) + i, 8, stride=2), :] = acc[RG * i + r]

        def values_mxu(g, chunks):
            acc = [None] * 3
            for c in chunks:
                if c in x_chunks:
                    p = lambda: get(lp, L_0 + c - nvc, g)
                else:
                    p0, p1 = (ps[c // cgran][2 * (c % cgran) + h] for h in range(2))
                    p01 = _rows8(jnp.where(sub == 0, p0, jnp.where(sub == 1, p1, 0.0)))
                    p = lambda: p01
                for t in range(3):
                    y = _mm(p(), _tile(vs, 24 * g + 8 * t, c))
                    acc[t] = y if acc[t] is None else acc[t] + y
                    tie(acc[t])
                    yield
            for t in range(3):
                accx[t] = jnp.where((sub & 1) == head[t], acc[t], 0.0)

        def finish_values(g, with_vpu=True):
            inv = 1.0 / jnp.sum(dens[g & 3], axis=-1, keepdims=True)
            inv0 = jnp.broadcast_to(inv[0:1], (8, 128))
            inv1 = jnp.broadcast_to(inv[1:2], (8, 128))
            for t in range(3):
                o = accx[t]
                if with_vpu:
                    blk = accs[pl.ds(pl.multiple_of(128 * t + 128 * (g >> 8), 128), 128), :]
                    o = o + jnp.sum(blk.T.reshape(16, 8, 128), axis=0)
                o = jnp.broadcast_to(jnp.sum(o, axis=0, keepdims=True), (8, 128))
                o = o * (inv0, jnp.where(head[1] == 1, inv1, inv0), inv1)[t]
                put(lo, L_0 + t, _rows16(o))
                tie(o, n_pbuf - 1)
                yield

        def project_o(g):
            acc = [xs[c + 8 * (g >> 8)] for c in range(ND)]
            for t in range(3):
                for c in range(ND):
                    acc[c] = acc[c] + _mm(get(lo, L_0 + t, g), _tile(wos, 24 * g + 8 * t, c))
                    tie(acc[c])
                    yield
            for c in range(ND):
                xs[c] = acc[c]

        def run(*gens):
            for gen in gens:
                for _ in gen:
                    pass

        def attend(g, with_o):
            s, q = [], []
            mxu = [(scores(g + 1, s), 3 * NC, lq), (project_q(jnp.minimum(g + 2, NG - 1), q), 3 * ND, lq),
                   (values_mxu(g, x_chunks), 3 * nx, lp)]
            if with_o:
                mxu.append((project_o(g - 1), 3 * ND, lo))
            step = (f1 - f0) / sum(n for _, n, _ in mxu)
            events, gens, pos = [], [], 0
            for gen, n, buf in mxu:
                events += [(f0 + step * (pos + k + 0.5), len(gens), buf) for k in range(n)]
                pos += n
                events.append((f0 + step * pos, len(gens), None))
                gens.append(gen)
            if with_o:
                events += [(ft0 + (ft1 - ft0) * (k + 0.5) / 3, len(gens), None) for k in range(3)]
                gens.append(finish_values(g - 1))
            n_units = 2 * (12 // RG) * n_pbuf
            events += [((k + 0.5) / n_units, len(gens), None) for k in range(n_units)] + [(2, len(gens), None)]
            events.sort(key=lambda ev: ev[:2])
            now = [0]

            def next_lhs():
                bufs = []
                for _, i, buf in events[now[0] + 1:]:
                    if i == len(gens) - 1:
                        break
                    if buf is not None and not any(buf is b for b in bufs):
                        bufs.append(buf)
                return bufs

            gens.append(values_vpu(g, next_lhs))
            unit[0] = 0
            for now[0], ev in enumerate(events):
                next(gens[ev[1]], None)
            unit[0] = None
            store_q(q)
            softmax(s, g + 1)

        def load_x():
            return jnp.concatenate([xs[c] for c in range(ND)], axis=1)

        def layer(l, _):
            first = pl.when(l == 0)
            z = l >> 8

            @first
            def _():
                wait(wq_cp())
                start(k_cp(1))
                start(v_cp(0))
                wait(k_cp(0))
                start(k_cp(2))
                start(v_cp(1))
            xc, rstd = _layernorm(load_x())
            xc = _rows16(xc)
            for kk in range(ND):
                put(lq, L_X + kk, xc[:, 128 * kk:128 * (kk + 1)])
            put(lq, L_RSTD, rstd)
            s, q0, q1 = [], [], []
            run(project_q(z, q0))
            store_q(q0)
            run(scores(z, s), project_q(z + 1, q1))
            softmax(s, 0)
            store_q(q1)

            @first
            def _():
                wait(wo_cp())
                wait(k_cp(1))
                wait(v_cp(0))
                start(k_cp(3))
                start(v_cp(2))
                prepare_v(0, x_chunks, e_chunks)
                retile_wo()
            attend(z, False)

            def pair(g, _):
                @first
                def _():
                    wait(k_cp(g + 1))
                    wait(v_cp(g))
                    pl.when(g + 3 < NG)(lambda: start(k_cp(g + 3)))
                    pl.when(g + 2 < NG)(lambda: start(v_cp(g + 2)))
                    pl.when(g + 3 == NG)(lambda: start(w13_cp()))
                    pl.when(g + 2 == NG)(lambda: start(w2_cp(0)))
                    prepare_v(g, x_chunks, e_chunks)
                attend(g, True)

            lax.fori_loop(1, NG - 1, pair, None)

            @first
            def _():
                wait(v_cp(NG - 1))
                start(w2_cp(1))
                prepare_v(NG - 1, x_chunks + v_chunks, [])
                wait(w13_cp())
            run(finish_values(z + NG - 2), values_mxu(z + NG - 1, x_chunks + v_chunks), project_o(z + NG - 2),
                finish_values(z + NG - 1, False), project_o(z + NG - 1))

            first(lambda: wait(w2_cp(0)))
            x = load_x()
            xc, rstd = _layernorm(x)
            xc = _rows16(xc)
            hs = []
            for c in range(F // 128):
                gate, up = (rstd * functools.reduce(jnp.add, [
                    _mm(xc[:, 128 * kk:128 * (kk + 1)], _tile(w, 8 * kk, c)) for kk in range(ND)])
                            for w in (w1s, w3s))
                hs.append(_rows16(gate * jax.nn.sigmoid(gate) * up))
            acc = [x[:, 128 * c:128 * (c + 1)] for c in range(ND)]
            for i, part in enumerate(w2_parts):
                if i:
                    first(lambda: wait(w2_cp(i)))
                for kk in range(*part):
                    for c in range(ND):
                        acc[c] = acc[c] + _mm(hs[kk], _tile(w2s, 8 * kk, c))
            for c in range(ND):
                xs[c] = acc[c]

        x = jnp.broadcast_to(x_ref[0].astype(F32), (8, D))
        for c in range(ND):
            xs[c] = x[:, 128 * c:128 * (c + 1)]
        lax.fori_loop(0, 2, layer, None)
        o_ref[0] = load_x()[0:1].astype(o_ref.dtype)

    def tiles(r, c):
        return pltpu.VMEM((r // 16, c // 128, 8, 128), I32)

    def vregs(n, dtype):
        return pltpu.VMEM((-(-n // 4) * 4, 8, 128), dtype)

    scratch = [
        tiles(H * DH, WINDOW), tiles(H * DH, WINDOW), pltpu.VMEM((NT - 24, ne, 8, 128), F32),
        tiles(D, H * DH), tiles(H * DH, D), tiles(D, F), tiles(D, F), tiles(F, D),
        vregs(ND, F32), vregs(L_RSTD + 1, I32), vregs(L_0 + 3, I32), vregs(L_0 + nx, I32),
        pltpu.VMEM((2 * DH, 128), F32), vregs(3, F32), vregs(4, F32), vregs(12, I32),
        pltpu.SemaphoreType.DMA((6,)),
    ] + [vregs(2 * cgran + 1, F32)] * n_pbuf + [pltpu.VMEM((1, 1, D), BF)]
    return kernel, scratch


def build(**schedule):
    def call(A_x, A_k_cache, A_v_cache, A_wq, A_wo, B_x, B_w1, B_w3, B_w2):
        def tile_view(w):
            return w.reshape(w.shape[0] // 16, 2, 8, w.shape[1] // 128, 128).transpose(0, 1, 3, 2, 4)

        def cache_view(c):
            return tile_view(c.transpose(0, 1, 3, 2).reshape(H * DH, SK))

        kernel, scratch = make_kernel(**schedule)
        return pl.pallas_call(
            kernel,
            out_shape=jax.ShapeDtypeStruct(A_x.shape, A_x.dtype),
            in_specs=[pl.BlockSpec(memory_space=pl.ANY)] * 8,
            out_specs=pl.BlockSpec(memory_space=pltpu.VMEM),
            scratch_shapes=scratch,
            compiler_params=pltpu.CompilerParams(vmem_limit_bytes=128 * 2**20),
            name="fused",
        )(A_x, cache_view(A_k_cache), cache_view(A_v_cache), tile_view(A_wq),
          tile_view(A_wo).reshape(NT, ND, 16, 128), tile_view(B_w1), tile_view(B_w3), tile_view(B_w2))
    return call


@jax.jit
def pallas_interleave_layers__sliding_block_cached__glu_gated_swiglu__decode_kernel(
    A_x: jax.Array,
    A_k_cache: jax.Array,
    A_v_cache: jax.Array,
    A_wq: jax.Array,
    A_wo: jax.Array,
    B_x: jax.Array,
    B_w1: jax.Array,
    B_w3: jax.Array,
    B_w2: jax.Array,
):
    return build()(A_x, A_k_cache, A_v_cache, A_wq, A_wo, B_x, B_w1, B_w3, B_w2)
```
